```python
import os as _os
_os.environ.setdefault("JAX_PLATFORMS", "cpu")
import jax
import jax.numpy as jnp

def _softmax(x, axis=-1):
    return jax.nn.softmax(x, axis=axis)
def _gelu(x):
    return jax.nn.gelu(x, approximate=True)
def _silu(x):
    return jax.nn.silu(x)
def _sigmoid(x):
    return jax.nn.sigmoid(x)
def _layernorm(x, axis=-1, eps=1e-5):
    m = jnp.mean(x, axis=axis, keepdims=True)
    v = jnp.var(x, axis=axis, keepdims=True)
    return (x - m) / jnp.sqrt(v + eps)
def _scatter_add(tgt, idx, src, axis=0):
    return tgt.at[idx].add(src)
def _segment_sum(src, seg, n):
    return jax.ops.segment_sum(src, seg, n)
class _Rng:
    def __init__(self, key):
        self._k = key
    def _next(self):
        self._k, sub = jax.random.split(self._k)
        return sub
    def normal(self, shape):
        return jax.random.normal(self._next(), shape, dtype=jnp.bfloat16)
    def randint(self, lo, hi, shape):
        return jax.random.randint(self._next(), shape, lo, hi, dtype=jnp.int32)
    def uniform(self, shape, lo=0.0, hi=1.0):
        return jax.random.uniform(self._next(), shape, jnp.bfloat16, lo, hi)
    def permutation(self, n):
        return jax.random.permutation(self._next(), n)


kernel_name = 'sequential_preLN__mha_block__dense_activation_squared_relu__prompt'

def setup_inputs():
    _rng = _Rng(jax.random.key(int.from_bytes(__import__("os").urandom(4), "little")))
    _w = (lambda a: (lambda t: t.astype(jnp.bfloat16) if jnp.issubdtype(t.dtype, jnp.floating) else t)(jnp.asarray(a)))
    def _A_setup():
        B, S, D, H = 1, 2048, 448, 16
        return {
            "x": _w((lambda *s: _rng.normal(s) * 0.05)(B, S, D)),
            "wqkv": _w((lambda *s: _rng.normal(s) * 0.05)(D, 3 * D)),
            "wo": _w((lambda *s: _rng.normal(s) * 0.05)(D, D)),
        }
    _A_in = _A_setup()

    def _B_setup():
        B, S, D, F = 1, 2048, 448, 1792
        return {
            "x": _w((lambda *s: _rng.normal(s) * 0.05)(B, S, D)),
            "w1": _w((lambda *s: _rng.normal(s) * 0.05)(D, F)),
            "b1": _w((lambda *s: _rng.normal(s) * 0.05)(F)),
            "w2": _w((lambda *s: _rng.normal(s) * 0.05)(F, D)),
            "b2": _w((lambda *s: _rng.normal(s) * 0.05)(D)),
        }
    _B_in = _B_setup()

    return {
        "A_x": _A_in["x"],
        "A_wqkv": _A_in["wqkv"],
        "A_wo": _A_in["wo"],
        "B_x": _B_in["x"],
        "B_w1": _B_in["w1"],
        "B_b1": _B_in["b1"],
        "B_w2": _B_in["w2"],
        "B_b2": _B_in["b2"],
    }

def reference(A_x, A_wqkv, A_wo, B_x, B_w1, B_b1, B_w2, B_b2):
    def _A_ref(x, wqkv, wo):
        B, S, D = x.shape
        H = 16
        Dh = D // H
        qkv = (lambda x, *d: x.transpose(*d))((x @ wqkv).reshape(B, S, 3, H, Dh), 2, 0, 3, 1, 4)
        q, k, v = qkv[0], qkv[1], qkv[2]
        scores = jnp.einsum("bhqd,bhkd->bhqk", q, k) * (Dh ** -0.5)
        p = _softmax(scores, axis=-1)
        o = jnp.einsum("bhqk,bhkd->bhqd", p, v)
        return (lambda x, *d: x.transpose(*d))(o, 0, 2, 1, 3).reshape(B, S, D) @ wo

    def _B_ref(x, w1, b1, w2, b2):
        h = jnp.einsum("bsd,df->bsf", x, w1) + b1
        zero = jnp.zeros_like(h)
        r = jnp.where(h > zero, h, zero)
        h = r * r
        out = jnp.einsum("bsf,fd->bsd", h, w2) + b2
        return out

    x = A_x
    h = x + _A_ref(_layernorm(x, axis=-1), A_wqkv, A_wo)
    h2 = h + _B_ref(_layernorm(h, axis=-1), B_w1, B_b1, B_w2, B_b2)
    return h2
```

```python
import functools, math
import jax, jax.numpy as jnp
from jax import lax
from jax.experimental import pallas as pl
from jax.experimental.pallas import tpu as pltpu

S, D, H, DH, F = 2048, 448, 16, 28, 1792
HP = 32
DP = H * HP
GW = 4 * DH
DA = D + 16
EPS = 1e-5
BF = jnp.bfloat16
F32 = jnp.float32

def _ln_t(xf):
    m = jnp.sum(xf, axis=0, keepdims=True) * (1.0 / D)
    c = xf - m
    v = jnp.sum(c * c, axis=0, keepdims=True) * (1.0 / D)
    return c * lax.rsqrt(v + EPS)

def _make(TQ=512, KC=128, RC=512, UH=5, B1D=True, PVFIRST=False):
    NQ = S // TQ
    NKC = S // KC
    NRC = S // RC
    qscale = (DH ** -0.5) * math.log2(math.e)
    assert (H - 1) % UH == 0

    def kernel(xt_hbm, wqkv_hbm, wo_hbm, w1_hbm, b1_ref, w2t_hbm, b2_ref, o_ref,
               xt, wqkv, wo, w1a, w2t, sems,
               wt_sc, tmp_sc, wot_sc, w1t_sc, b2c_sc,
               qt_sc, k_sc, vt_sc, s_sc, m_sc, ot_sc):
        t = pl.program_id(0)
        rowi = lax.broadcasted_iota(jnp.int32, (GW, TQ), 0)

        def qmask(h, qoff):
            g = h // 4
            j = h % 4
            r0 = g * GW
            if not isinstance(r0, int):
                r0 = pl.multiple_of(r0, 16)
            q = qt_sc[pl.ds(r0, GW), pl.ds(qoff, TQ)]
            return jnp.where((rowi >= j * DH) & (rowi < (j + 1) * DH), q, jnp.zeros_like(q)), g

        def qk_chunk(qm, g, c):
            s = jnp.dot(k_sc[g, c * KC:(c + 1) * KC, :], qm, preferred_element_type=F32)
            s_sc[c * KC:(c + 1) * KC, :] = s
            return jnp.max(s.reshape(KC // 8, 8, TQ), axis=0)

        def p_chunk(c, m):
            return jnp.exp2(s_sc[c * KC:(c + 1) * KC, :] - m).astype(BF)

        def pv_chunk(h, c, p):
            r0 = h * HP
            if not isinstance(r0, int):
                r0 = pl.multiple_of(r0, HP)
            v = vt_sc[pl.ds(r0, HP), c * KC:(c + 1) * KC]
            return jnp.dot(v, p, preferred_element_type=F32)

        def stage(h_next, qoff_next, h_cur, m_cur):
            mn = None
            o = None
            qm, g = qmask(h_next, qoff_next)
            for c in range(NKC):
                if h_cur is not None:
                    p = p_chunk(c, m_cur)
                if PVFIRST and h_cur is not None:
                    oc = pv_chunk(h_cur, c, p)
                    o = oc if o is None else o + oc
                mc = qk_chunk(qm, g, c)
                mn = mc if mn is None else jnp.maximum(mn, mc)
                if not PVFIRST and h_cur is not None:
                    oc = pv_chunk(h_cur, c, p)
                    o = oc if o is None else o + oc
            if h_cur is not None:
                l = o[DH:DH + 1, :]
                r = pl.reciprocal(l, approx=True)
                r = r * (2.0 - l * r)
                r0 = h_cur * HP
                if not isinstance(r0, int):
                    r0 = pl.multiple_of(r0, HP)
                ot_sc[pl.ds(r0, HP), :] = (o * r).astype(BF)
            return jnp.max(mn, axis=0, keepdims=True)

        @pl.when(t == 0)
        def _():
            cp_w = pltpu.make_async_copy(wqkv_hbm, wqkv, sems.at[0])
            cp_x0 = pltpu.make_async_copy(xt_hbm.at[:, 0:RC], xt.at[:, 0:RC], sems.at[1])
            cp_x1 = pltpu.make_async_copy(xt_hbm.at[:, RC:S], xt.at[:, RC:S], sems.at[2])
            cp_wo = pltpu.make_async_copy(wo_hbm, wo, sems.at[3])
            cp_w1 = pltpu.make_async_copy(w1_hbm, w1a.at[0:D, :], sems.at[4])
            cp_w2 = pltpu.make_async_copy(w2t_hbm, w2t, sems.at[5])
            cp_w.start(); cp_x0.start(); cp_x1.start()
            cp_w.wait(); cp_x0.wait()
            cp_wo.start(); cp_w1.start(); cp_w2.start()
            wt_sc[0:2 * D, :] = wqkv[:, 0:2 * D].T
            tmp_sc[...] = wqkv[:, 2 * D:3 * D].astype(F32).T
            zpad = jnp.zeros((HP - DH, D), F32)
            for h in range(H):
                blk = jnp.concatenate([tmp_sc[h * DH:(h + 1) * DH, :], zpad], axis=0)
                wt_sc[2 * D + h * HP:2 * D + (h + 1) * HP, :] = blk.astype(BF)

            def proj(c):
                c0 = c * RC
                xn = _ln_t(xt[:, pl.ds(c0, RC)].astype(F32)).astype(BF)
                qkv = jnp.dot(wt_sc[...], xn, preferred_element_type=F32)
                qt_sc[:, pl.ds(c0, RC)] = (qkv[0:D] * qscale).astype(BF)
                for g in range(4):
                    kt = qkv[D + g * GW:D + (g + 1) * GW].astype(BF)
                    k_sc[g, pl.ds(c0, RC), :] = kt.T
                vt = qkv[2 * D:]
                row = lax.broadcasted_iota(jnp.int32, vt.shape, 0)
                vt = jnp.where(row % HP == DH, 1.0, vt)
                vt_sc[:, pl.ds(c0, RC)] = vt.astype(BF)

            proj(0)
            cp_x1.wait()
            proj(1)
            cp_wo.wait(); cp_w1.wait(); cp_w2.wait()
            for c in range(2, NRC):
                proj(c)
            tmp_sc[...] = wo[...].astype(F32)
            blks = []
            for h in range(H):
                blks.append(tmp_sc[h * DH:(h + 1) * DH, :])
                blks.append(zpad)
            wot_sc[...] = jnp.concatenate(blks, axis=0).astype(BF).T
            r16 = lax.broadcasted_iota(jnp.int32, (16, F), 0)
            b1 = b1_ref[...].astype(F32).reshape(1, F)
            w1a[D:DA, :] = jnp.where(r16 == 0, b1, 0.0).astype(BF)
            w1t_sc[...] = w1a[...].T
            b2 = b2_ref[...].astype(F32).reshape(1, D)
            b2c_sc[...] = jnp.broadcast_to(b2, (128, D)).T
            m_sc[...] = stage(0, 0, None, None)

        q0 = pl.multiple_of(t * TQ, TQ)

        def body(i, m):
            h = UH * i
            for u in range(UH):
                m = stage(h + u + 1, q0, h + u, m)
            return m
        m = lax.fori_loop(0, (H - 1) // UH, body, m_sc[...])
        qn = pl.multiple_of(jnp.minimum(t + 1, NQ - 1) * TQ, TQ)
        m_sc[...] = stage(0, qn, H - 1, m)

        x = xt[:, pl.ds(q0, TQ)].astype(F32)
        h1 = x + jnp.dot(wot_sc[...], ot_sc[...], preferred_element_type=F32)
        hn = _ln_t(h1).astype(BF)
        r16 = lax.broadcasted_iota(jnp.int32, (16, TQ), 0)
        hna = jnp.concatenate([hn, jnp.where(r16 == 0, 1.0, 0.0).astype(BF)], axis=0)
        u = jnp.dot(w1t_sc[...], hna, preferred_element_type=F32)
        u = jnp.maximum(u, 0.0)
        u = (u * u).astype(BF)
        y = jnp.dot(w2t[...], u, preferred_element_type=F32)
        b2c = jnp.concatenate([b2c_sc[...]] * (TQ // 128), axis=1)
        o_ref[...] = (h1 + y + b2c).astype(o_ref.dtype)

    def fn(A_x, A_wqkv, A_wo, B_x, B_w1, B_b1, B_w2, B_b2):
        xt = A_x.reshape(S, D).T
        w2t = B_w2.T
        anyspec = pl.BlockSpec(memory_space=pl.ANY)
        full = lambda shp: pl.BlockSpec(shp, lambda t: (0,) * len(shp))
        if B1D:
            b1, b2 = B_b1, B_b2
        else:
            b1, b2 = B_b1.reshape(1, F), B_b2.reshape(1, D)
        out = pl.pallas_call(
            kernel,
            grid=(NQ,),
            in_specs=[anyspec, anyspec, anyspec, anyspec, full(b1.shape), anyspec, full(b2.shape)],
            out_specs=pl.BlockSpec((D, TQ), lambda t: (0, t)),
            out_shape=jax.ShapeDtypeStruct((D, S), BF),
            scratch_shapes=[
                pltpu.VMEM((D, S), BF), pltpu.VMEM((D, 3 * D), BF), pltpu.VMEM((D, D), BF),
                pltpu.VMEM((DA, F), BF), pltpu.VMEM((D, F), BF), pltpu.SemaphoreType.DMA((6,)),
                pltpu.VMEM((2 * D + DP, D), BF), pltpu.VMEM((D, D), F32), pltpu.VMEM((D, DP), BF),
                pltpu.VMEM((F, DA), BF), pltpu.VMEM((D, 128), F32),
                pltpu.VMEM((D, S), BF), pltpu.VMEM((4, S, GW), BF), pltpu.VMEM((DP, S), BF),
                pltpu.VMEM((S, TQ), F32), pltpu.VMEM((1, TQ), F32), pltpu.VMEM((DP, TQ), BF)],
            compiler_params=pltpu.CompilerParams(dimension_semantics=("arbitrary",), vmem_limit_bytes=100 * 1024 * 1024),
        )(xt, A_wqkv, A_wo, B_w1, b1, w2t, b2)
        return out.T.reshape(1, S, D)
    return fn


_fn = _make()


@jax.jit
def pallas_sequential_preLN__mha_block__dense_activation_squared_relu__prompt_kernel(
    A_x: jax.Array,
    A_wqkv: jax.Array,
    A_wo: jax.Array,
    B_x: jax.Array,
    B_w1: jax.Array,
    B_b1: jax.Array,
    B_w2: jax.Array,
    B_b2: jax.Array,
):
    return _fn(A_x, A_wqkv, A_wo, B_x, B_w1, B_b1, B_w2, B_b2)
```

```python
import functools, math
import jax, jax.numpy as jnp
from jax import lax
from jax.experimental import pallas as pl
from jax.experimental.pallas import tpu as pltpu

S, D, H, DH, F = 2048, 448, 16, 28, 1792
HP = 32
DP = H * HP
GW = 4 * DH
DA = D + 16
EPS = 1e-5
BF = jnp.bfloat16
F32 = jnp.float32

class _NullScope:
    def __init__(self, *a): pass
    def __enter__(self): return self
    def __exit__(self, *a): return False

def _ln_t(xf):
    m = jnp.sum(xf, axis=0, keepdims=True) * (1.0 / D)
    c = xf - m
    v = jnp.sum(c * c, axis=0, keepdims=True) * (1.0 / D)
    return c * lax.rsqrt(v + EPS)

def _mo(x, m):
    return x if isinstance(x, int) else pl.multiple_of(x, m)

U32 = jnp.uint32

def _pk(x):
    return pltpu.bitcast(x, U32)

def _up(x):
    return pltpu.bitcast(x, BF)

def _dot(a, b):
    return jnp.dot(a, b, preferred_element_type=F32)

def _make(TQ=512, KC=128, RC=512, UH=7, L=1, SCOPE=False, TAIL=1, VC=True, NB=2, LW=128, FILL=2, HOLD=3, PK=True, EXTRA=1):
    NQ = S // TQ
    NKC = S // KC
    NRC = S // RC
    RS = 2 * NKC
    NA = (H - 1) % UH
    NIT = (H - 1) // UH
    qscale = (DH ** -0.5) * math.log2(math.e)
    scope = jax.named_scope if SCOPE else _NullScope
    WR = 3 * D if VC else 2 * D + DP

    def shifts(n):
        base = [RS // n] * n
        base[0] += RS - sum(base)
        assert all(L <= b <= NKC for b in base), base
        return base

    def kernel(xt_hbm, wqkv_hbm, wo_hbm, w1_hbm, b1_hbm, w2t_hbm, b2_hbm, o_ref,
               xt, wqkv, wo, w1a, w2t, b1v, b2v, sems,
               wt_sc, tmp_sc, wot_sc, w1t_sc, b2c_sc, xn_sc,
               qt_sc, k_sc, vt_sc, s_sc, ot_sc):
        t = pl.program_id(0)
        q0 = pl.multiple_of(t * TQ, TQ)
        rowi = lax.broadcasted_iota(jnp.int32, (GW // 2, TQ), 0)

        def qmask(h):
            g = h // 4
            j = h % 4
            q = qt_sc[pl.ds(_mo(g * (GW // 2), 8), GW // 2), pl.ds(q0, TQ)]
            hd = DH // 2
            return _up(jnp.where((rowi >= j * hd) & (rowi < (j + 1) * hd), q, jnp.zeros_like(q))), g

        def qk_chunk(qm, g, c, slot):
            s = _dot(_up(k_sc[g, c * KC // 2:(c + 1) * KC // 2, :]), qm)
            s_sc[slot * KC:(slot + 1) * KC, :] = s
            return jnp.max(s.reshape(KC // 8, 8, TQ), axis=0)

        def p_chunk(slot, m):
            return jnp.exp2(s_sc[slot * KC:(slot + 1) * KC, :] - m).astype(BF)

        def pv_chunk(h, c, p):
            v = _up(vt_sc[pl.ds(_mo(h * (HP // 2), HP // 2), HP // 2), c * KC:(c + 1) * KC])
            return _dot(v, p)

        def finish(h, o):
            l = o[DH:DH + 1, :]
            r = pl.reciprocal(l, approx=True)
            r = r * (2.0 - l * r)
            ot_sc[pl.ds(_mo(h * (HP // 2), HP // 2), HP // 2), :] = _pk((o * r).astype(BF))

        def run(cur, nxt, m0, filler=None):
            n_st = len(nxt)
            off = [0]
            if n_st > 1:
                for sft in shifts(n_st):
                    off.append((off[-1] - sft) % RS)
            else:
                off.append(0)
            assert off[-1] == 0
            ms = {0: m0}
            mrun, oacc, qms, pv_at = {}, {}, {}, {}
            for j in range(n_st * NKC):
                if cur[j // NKC] is not None:
                    pv_at.setdefault(j if j < NKC else j + L, []).append(j)
            last = max(list(pv_at) + [n_st * NKC - 1])
            for n in range(last + 1):
                ps = []
                for j in pv_at.get(n, []):
                    u, c = divmod(j, NKC)
                    ps.append((u, c, p_chunk((off[u] + c) % RS, ms[u])))
                if n < n_st * NKC and nxt[n // NKC] is not None:
                    u, c = divmod(n, NKC)
                    if c == 0:
                        qms[u] = qmask(nxt[u])
                    mc = qk_chunk(qms[u][0], qms[u][1], c, (off[u + 1] + c) % RS)
                    mrun[u] = mc if c == 0 else jnp.maximum(mrun[u], mc)
                    if c == NKC - 1:
                        ms[u + 1] = jnp.max(mrun[u], axis=0, keepdims=True)
                if filler is not None:
                    filler(n)
                for (u, c, p) in ps:
                    oc = pv_chunk(cur[u], c, p)
                    oacc[u] = oc if c == 0 else oacc[u] + oc
                    if c == NKC - 1:
                        finish(cur[u], oacc[u])
            return ms.get(n_st)

        @pl.when(t == 0)
        def _():
          with scope('prologue'):
            cp_w = pltpu.make_async_copy(wqkv_hbm, wqkv, sems.at[0])
            cp_x0 = pltpu.make_async_copy(xt_hbm.at[:, 0:RC], xt.at[:, 0:RC], sems.at[1])
            cp_x1 = pltpu.make_async_copy(xt_hbm.at[:, RC:S], xt.at[:, RC:S], sems.at[2])
            cp_wo = pltpu.make_async_copy(wo_hbm, wo, sems.at[3])
            cp_w1 = pltpu.make_async_copy(w1_hbm, w1a.at[0:D, :], sems.at[4])
            cp_w2 = pltpu.make_async_copy(w2t_hbm, w2t, sems.at[5])
            cp_b1 = pltpu.make_async_copy(b1_hbm, b1v, sems.at[6])
            cp_b2 = pltpu.make_async_copy(b2_hbm, b2v, sems.at[7])
            cp_x0.start(); cp_w.start(); cp_x1.start()

            def ln1(c):
                for j in range(c * RC // LW, (c + 1) * RC // LW):
                    xn_sc[:, j * LW:(j + 1) * LW] = _pk(_ln_t(xt[:, j * LW:(j + 1) * LW].astype(F32)).astype(BF))

            def proj_k(c):
                cs = slice(c * RC, (c + 1) * RC)
                kt = _dot(_up(wt_sc[D // 2:D, :]), _up(xn_sc[:, cs]))
                for g in range(4):
                    k_sc[g, c * RC // 2:(c + 1) * RC // 2, :] = _pk(kt[g * GW:(g + 1) * GW].astype(BF).T)

            def proj_q(c):
                cs = slice(c * RC, (c + 1) * RC)
                q = _dot(_up(wt_sc[0:D // 2, :]), _up(xn_sc[:, cs]))
                qt_sc[:, cs] = _pk((q * qscale).astype(BF))

            def proj_qk(c):
                proj_k(c)
                proj_q(c)

            def proj_v(c):
                cs = slice(c * RC, (c + 1) * RC)
                vt = _dot(_up(wt_sc[D:3 * D // 2, :]), _up(xn_sc[:, cs]))
                r4 = lax.broadcasted_iota(jnp.int32, (HP - DH, RC), 0)
                pad = jnp.where(r4 == 0, 1.0, 0.0)
                for h in range(H):
                    blk = jnp.concatenate([vt[h * DH:(h + 1) * DH], pad], axis=0)
                    vt_sc[h * HP // 2:(h + 1) * HP // 2, cs] = _pk(blk.astype(BF))

            with scope('wait0'):
                cp_x0.wait()
            ln1(0)
            with scope('wait0b'):
                cp_w.wait()
            cp_wo.start(); cp_w1.start(); cp_w2.start(); cp_b1.start(); cp_b2.start()
            zpad = jnp.zeros((HP - DH, D), F32)
            if VC:
                wt_sc[...] = _pk(wqkv[...].T)
            else:
                wt_sc[0:2 * D, :] = wqkv[:, 0:2 * D].T
                tmp_sc[...] = wqkv[:, 2 * D:3 * D].astype(F32).T
                for h in range(H):
                    blk = jnp.concatenate([tmp_sc[h * DH:(h + 1) * DH, :], zpad], axis=0)
                    wt_sc[2 * D + h * HP:2 * D + (h + 1) * HP, :] = blk.astype(BF)
            proj_qk(0)
            cp_x1.wait()
            proj_v(0)
            ln1(1)
            proj_qk(1)
            ln1(2)
            proj_v(1)
            cp_wo.wait(); cp_w1.wait(); cp_w2.wait(); cp_b1.wait(); cp_b2.wait()
            proj_qk(2)
            ln1(3)
            proj_v(2)
            proj_qk(3)
            proj_v(3)
            tmp_sc[...] = wo[...].astype(F32)
            blks = []
            for h in range(H):
                blks.append(tmp_sc[h * DH:(h + 1) * DH, :])
                blks.append(zpad)
            wot_sc[...] = _pk(jnp.concatenate(blks, axis=0).astype(BF).T)
            r16 = lax.broadcasted_iota(jnp.int32, (16, F), 0)
            b1 = b1v[...].astype(F32).reshape(1, F)
            w1a[D:DA, :] = jnp.where(r16 == 0, b1, 0.0).astype(BF)
            w1t_sc[...] = _pk(w1a[...].T)
            b2 = b2v[...].astype(F32).reshape(1, D)
            b2c_sc[...] = jnp.broadcast_to(b2, (128, D)).T

        with scope('headA'):
            m = run([None] + list(range(NA)), list(range(NA + 1)), None)

        def body(i, m):
            h = NA + UH * i
            return run([h + u for u in range(UH)], [h + u + 1 for u in range(UH)], m)
        with scope('headloop'):
            m = lax.fori_loop(0, NIT, body, m)

        TB = TQ // NB
        KS = DP - 128
        RB = 64
        NRB = D // RB
        part = {}

        def wo_part(b, rb):
            part[(b, rb)] = _dot(_up(wot_sc[rb * RB // 2:(rb + 1) * RB // 2, 0:KS]), _up(ot_sc[0:KS // 2, b * TB:(b + 1) * TB]))

        if TAIL == 0:
            run([H - 1], [None], m)
            att = [_dot(_up(wot_sc[...]), _up(ot_sc[:, b * TB:(b + 1) * TB])) for b in range(NB)]
        else:
            todo = [(b, rb) for b in range(NB) for rb in range(NRB)]

            def filler(n):
                if n % FILL == 0 and len(todo) > NRB * NB // 2 - EXTRA:
                    wo_part(*todo.pop(0))
            run([H - 1], [None], m, filler)
            while len(todo) > NRB * NB // 2 - HOLD and todo:
                wo_part(*todo.pop(0))
            att = []
            for b in range(NB):
                while todo and todo[0][0] <= b:
                    wo_part(*todo.pop(0))
                lastk = _dot(_up(wot_sc[:, KS:DP]), _up(ot_sc[KS // 2:DP // 2, b * TB:(b + 1) * TB]))
                att.append(jnp.concatenate([part[(b, rb)] for rb in range(NRB)], axis=0) + lastk)

        r16 = lax.broadcasted_iota(jnp.int32, (16, TB), 0)
        ones_row = jnp.where(r16 == 0, 1.0, 0.0).astype(BF)
        b2c = jnp.concatenate([b2c_sc[...]] * (TB // 128), axis=1)
        h1s, us = [], []
        for b in range(NB):
            x = xt[:, pl.ds(q0 + b * TB, TB)].astype(F32)
            h1 = x + att[b]
            h1s.append(h1)
            hna = jnp.concatenate([_ln_t(h1).astype(BF), ones_row], axis=0)
            u = jnp.maximum(_dot(_up(w1t_sc[...]), hna), 0.0)
            us.append((u * u).astype(BF))
        for b in range(NB):
            y = _dot(w2t[...], us[b])
            o_ref[:, b * TB:(b + 1) * TB] = (h1s[b] + y + b2c).astype(o_ref.dtype)

    def fn(A_x, A_wqkv, A_wo, B_x, B_w1, B_b1, B_w2, B_b2):
        xt = A_x.reshape(S, D).T
        w2t = B_w2.T
        anyspec = pl.BlockSpec(memory_space=pl.ANY)
        out = pl.pallas_call(
            kernel,
            grid=(NQ,),
            in_specs=[anyspec] * 7,
            out_specs=pl.BlockSpec((D, TQ), lambda t: (0, t)),
            out_shape=jax.ShapeDtypeStruct((D, S), BF),
            scratch_shapes=[
                pltpu.VMEM((D, S), BF), pltpu.VMEM((D, 3 * D), BF), pltpu.VMEM((D, D), BF),
                pltpu.VMEM((DA, F), BF), pltpu.VMEM((D, F), BF), pltpu.VMEM((F,), BF), pltpu.VMEM((D,), BF),
                pltpu.SemaphoreType.DMA((8,)),
                pltpu.VMEM((WR // 2, D), U32), pltpu.VMEM((D, D), F32), pltpu.VMEM((D // 2, DP), U32),
                pltpu.VMEM((F // 2, DA), U32), pltpu.VMEM((D, 128), F32), pltpu.VMEM((D // 2, S), U32),
                pltpu.VMEM((D // 2, S), U32), pltpu.VMEM((4, S // 2, GW), U32), pltpu.VMEM((DP // 2, S), U32),
                pltpu.VMEM((RS * KC, TQ), F32), pltpu.VMEM((DP // 2, TQ), U32)],
            compiler_params=pltpu.CompilerParams(dimension_semantics=("arbitrary",), vmem_limit_bytes=100 * 1024 * 1024),
        )(xt, A_wqkv, A_wo, B_w1, B_b1, w2t, B_b2)
        return out.T.reshape(1, S, D)
    return fn


_fn = _make()


@jax.jit
def pallas_sequential_preLN__mha_block__dense_activation_squared_relu__prompt_kernel(
    A_x: jax.Array,
    A_wqkv: jax.Array,
    A_wo: jax.Array,
    B_x: jax.Array,
    B_w1: jax.Array,
    B_b1: jax.Array,
    B_w2: jax.Array,
    B_b2: jax.Array,
):
    return _fn(A_x, A_wqkv, A_wo, B_x, B_w1, B_b1, B_w2, B_b2)
```

```python
import functools, math
import jax, jax.numpy as jnp
from jax import lax
from jax.experimental import pallas as pl
from jax.experimental.pallas import tpu as pltpu

S, D, H, DH, F = 2048, 448, 16, 28, 1792
HP = 32
DP = H * HP
GW = 4 * DH
DA = 512
EPS = 1e-5
BF = jnp.bfloat16
F32 = jnp.float32

class _NullScope:
    def __init__(self, *a): pass
    def __enter__(self): return self
    def __exit__(self, *a): return False

def _ln_t(xf):
    m = jnp.sum(xf, axis=0, keepdims=True) * (1.0 / D)
    c = xf - m
    v = jnp.sum(c * c, axis=0, keepdims=True) * (1.0 / D)
    return c * lax.rsqrt(v + EPS)

def _ln_stream(x1, x2, x3):
    m = jnp.sum(x1, axis=0, keepdims=True) * (1.0 / D)
    c = x2 - m
    v = jnp.sum(c * c, axis=0, keepdims=True) * (1.0 / D)
    return (x3 - m) * lax.rsqrt(v + EPS)

def _mo(x, m):
    return x if isinstance(x, int) else pl.multiple_of(x, m)

U32 = jnp.uint32

def _pk(x):
    return pltpu.bitcast(x, U32)

def _up(x):
    return pltpu.bitcast(x, BF)

def _acombos(a11, a12, a21, a22):
    return [a11 + a22, a21 + a22, a11, a22, a11 + a12, a21 - a11, a12 - a22]

def _dot(a, b):
    return jnp.dot(a, b, preferred_element_type=F32)

def _make(TQ=512, KC=128, RC=512, UH=7, L=1, SCOPE=False, TAIL=1, VC=True, NB=2, LW=128, FILL=2, HOLD=3, PK=True, EXTRA=1, ST1=True, ST2=True, TOK=True, WB=32, LNT=True, W1T=True, W1F=0.9, LNS=True, TS=32, LB=64, HS=True, WQT=True, WQ0=0.3, WQ1=0.9, NPRE=2, EARLY=False):
    NQ = S // TQ
    NKC = S // KC
    NRC = S // RC
    RS = 2 * NKC
    NA = (H - 1) % UH
    NIT = (H - 1) // UH
    qscale = (DH ** -0.5) * math.log2(math.e)
    scope = jax.named_scope if SCOPE else _NullScope
    WR = 3 * D if VC else 2 * D + DP

    def shifts(n):
        base = [RS // n] * n
        base[0] += RS - sum(base)
        assert all(L <= b <= NKC for b in base), base
        return base

    def kernel(xt_hbm, wqkv_hbm, wo_hbm, w1_hbm, b1_hbm, w2t_hbm, b2_hbm, o_ref,
               xt, wqkv, wo, w1a, w2t, b1v, b2v, sems,
               wt_sc, tmp_sc, wot_sc, w1s_sc, w2s_sc, b2c_sc, wq_sc,
               qt_sc, k_sc, vt_sc, s_sc, ot_sc, ha_sc, hb_sc):
        h_sc = (ha_sc, hb_sc)
        t = pl.program_id(0)
        q0 = pl.multiple_of(t * TQ, TQ)
        zs = [jnp.minimum(t, 0) * 128, jnp.minimum(t, 0) * 256]
        rowi = lax.broadcasted_iota(jnp.int32, (GW // 2, TQ), 0)

        rt_true = lax.broadcasted_iota(jnp.int32, (8, 128), 1) > (t - 100)

        def tie(v, tok):
            if tok is None:
                return v
            n = v.shape[0]
            return jnp.where(rt_true[None], v.reshape(n // 8, 8, 128), tok[None]).reshape(n, 128)

        def ln_paced(rd, put, tk, s1=None):
            nb = D // LB
            if s1 is None:
                for b in range(nb):
                    v = jnp.sum(tie(rd(0, b * LB, LB), next(tk)).reshape(LB // 8, 8, 128), axis=0)
                    s1 = v if s1 is None else s1 + v
            m8 = jnp.broadcast_to(jnp.sum(s1, axis=0, keepdims=True) * (1.0 / D), (8, 128))
            s2 = None
            for b in range(nb):
                c = rd(1, b * LB, LB).reshape(LB // 8, 8, 128) - tie(m8, next(tk))[None]
                v = jnp.sum(c * c, axis=0)
                s2 = v if s2 is None else s2 + v
            r = lax.rsqrt(jnp.sum(s2, axis=0, keepdims=True) * (1.0 / D) + EPS)
            for b in range(nb):
                c = rd(2, b * LB, LB).reshape(LB // 8, 8, 128) - tie(m8, next(tk))[None]
                put(b * LB, LB, c.reshape(LB, 128) * r)

        def spread(lst, n):
            if lst is None:
                return iter([None] * n)
            return iter([lst[(i * len(lst)) // n] for i in range(n)])

        def qmask(h):
            g = h // 4
            j = h % 4
            q = qt_sc[pl.ds(_mo(g * (GW // 2), 8), GW // 2), pl.ds(q0, TQ)]
            hd = DH // 2
            return _up(jnp.where((rowi >= j * hd) & (rowi < (j + 1) * hd), q, jnp.zeros_like(q))), g

        def qk_chunk(qm, g, c, slot):
            s = _dot(_up(k_sc[g, c * KC // 2:(c + 1) * KC // 2, :]), qm)
            s_sc[slot * KC:(slot + 1) * KC, :] = s
            return jnp.max(s.reshape(KC // 8, 8, TQ), axis=0)

        def p_chunk(slot, m):
            return jnp.exp2(s_sc[slot * KC:(slot + 1) * KC, :] - m).astype(BF)

        def pv_chunk(h, c, p):
            v = _up(vt_sc[pl.ds(_mo(h * (HP // 2), HP // 2), HP // 2), c * KC:(c + 1) * KC])
            return _dot(v, p)

        def finish(h, o):
            l = o[DH:DH + 1, :]
            r = pl.reciprocal(l, approx=True)
            r = r * (2.0 - l * r)
            ot_sc[pl.ds(_mo(h * (HP // 2), HP // 2), HP // 2), :] = _pk((o * r).astype(BF))

        def run(cur, nxt, m0, filler=None):
            n_st = len(nxt)
            off = [0]
            if n_st > 1:
                for sft in shifts(n_st):
                    off.append((off[-1] - sft) % RS)
            else:
                off.append(0)
            assert off[-1] == 0
            ms = {0: m0}
            mrun, oacc, qms, pv_at = {}, {}, {}, {}
            for j in range(n_st * NKC):
                if cur[j // NKC] is not None:
                    pv_at.setdefault(j if j < NKC else j + L, []).append(j)
            last = max(list(pv_at) + [n_st * NKC - 1])
            for n in range(last + 1):
                ps = []
                for j in pv_at.get(n, []):
                    u, c = divmod(j, NKC)
                    ps.append((u, c, p_chunk((off[u] + c) % RS, ms[u])))
                if n < n_st * NKC and nxt[n // NKC] is not None:
                    u, c = divmod(n, NKC)
                    if c == 0:
                        qms[u] = qmask(nxt[u])
                    mc = qk_chunk(qms[u][0], qms[u][1], c, (off[u + 1] + c) % RS)
                    mrun[u] = mc if c == 0 else jnp.maximum(mrun[u], mc)
                    if c == NKC - 1:
                        ms[u + 1] = jnp.max(mrun[u], axis=0, keepdims=True)
                if filler is not None:
                    filler(n)
                for (u, c, p) in ps:
                    oc = pv_chunk(cur[u], c, p)
                    oacc[u] = oc if c == 0 else oacc[u] + oc
                    if c == NKC - 1:
                        finish(cur[u], oacc[u])
            return ms.get(n_st)

        @pl.when(t == 0)
        def _():
          with scope('prologue'):
            cp_wb = pltpu.make_async_copy(wqkv_hbm.at[DA // 2:D, :], wqkv.at[DA // 2:D, :], sems.at[0])
            cp_wa = pltpu.make_async_copy(wqkv_hbm.at[0:DA // 2, :], wqkv.at[0:DA // 2, :], sems.at[8])
            cp_x0 = pltpu.make_async_copy(xt_hbm.at[:, 0:RC], xt.at[:, 0:RC], sems.at[1])
            cp_x1 = pltpu.make_async_copy(xt_hbm.at[:, RC:S], xt.at[:, RC:S], sems.at[2])
            cp_wo = pltpu.make_async_copy(wo_hbm, wo, sems.at[3])
            cp_w1 = pltpu.make_async_copy(w1_hbm, w1a.at[0:D, :], sems.at[4])
            cp_w2 = pltpu.make_async_copy(w2t_hbm, w2t, sems.at[5])
            cp_b1 = pltpu.make_async_copy(b1_hbm, b1v, sems.at[6])
            cp_b2 = pltpu.make_async_copy(b2_hbm, b2v, sems.at[7])
            cp_x0.start(); cp_wb.start(); cp_wa.start(); cp_x1.start()
            if EARLY:
                cp_wo.start(); cp_w1.start(); cp_w2.start(); cp_b1.start(); cp_b2.start()

            HB = RC // 2
            KH = DA // 2
            K2 = D - KH
            QH = D // 2
            MH = D + QH
            R_A, R_B = NRC * D, NRC * D + MH
            assert R_B + MH <= RS * KC and RC == TQ

            def ln1(c, tk=None):
                it = spread(tk, 4 * 3 * (D // LB))
                for j in range(RC // 128):
                    c0 = c * RC + j * 128

                    def rd(p, r0, n):
                        cc = c0 if (p == 0 or tk is None) else pl.multiple_of(c0 + zs[p - 1], 128)
                        return xt[r0:r0 + n, pl.ds(cc, 128)].astype(F32)

                    def put(r0, n, y):
                        s_sc[c * D + r0:c * D + r0 + n, j * 128:(j + 1) * 128] = y
                    ln_paced(rd, put, it)

            toks = []
            ctoks = {c: [] for c in range(NRC)}

            def wrows(i, lanes):
                if i == 0:
                    return jnp.concatenate([wt_sc[D // 2:D, lanes], wt_sc[0:QH // 2, lanes]], axis=0)
                return jnp.concatenate([wt_sc[D:3 * D // 2, lanes], wt_sc[QH // 2:D // 2, lanes]], axis=0)

            src0 = {0: lambda r: D // 2 + r if r < D // 2 else r - D // 2,
                    1: lambda r: D + r if r < D // 2 else QH // 2 + r - D // 2}

            def wblk(i, r, lanes):
                return _up(wt_sc[src0[i](r):src0[i](r) + 16, lanes]).astype(F32)

            def wq_combo7():
                for r in range(0, MH // 2, 16):
                    v = wblk(0, r, slice(KH, D)) - wblk(1, r, slice(KH, D))
                    wq_sc[4, r:r + 16, 0:K2] = _pk(v.astype(BF))

            def wq_combos(tk):
                it = spread(tk, 2 * (MH // 32))
                z = jnp.zeros((32, KH - K2), F32)
                for r in range(0, MH // 2, 16):
                    for lt in range(2):
                        tok = next(it)
                        ls = slice(lt * 128, (lt + 1) * 128)
                        a11, a21 = tie(wblk(0, r, ls), tok), tie(wblk(1, r, ls), tok)
                        if lt == 0:
                            a12, a22 = wblk(0, r, slice(KH, KH + 128)), wblk(1, r, slice(KH, KH + 128))
                        else:
                            a12 = jnp.concatenate([wblk(0, r, slice(KH + 128, D)), z], axis=1)
                            a22 = jnp.concatenate([wblk(1, r, slice(KH + 128, D)), z], axis=1)
                        for n, v in enumerate([a11 + a22, a21 + a22, a11 + a12, a21 - a11]):
                            wq_sc[n, r:r + 16, ls] = _pk(v.astype(BF))

            def fin_top(c, j, v):
                c0 = c * RC + j * HB
                for g in range(4):
                    k_sc[g, c0 // 2:(c0 + HB) // 2, :] = _pk(v[g * GW:(g + 1) * GW].astype(BF).T)
                qt_sc[0:QH // 2, c0:c0 + HB] = _pk((v[D:MH] * qscale).astype(BF))

            def fin_bot(c, j, v):
                c0 = c * RC + j * HB
                r4 = lax.broadcasted_iota(jnp.int32, (HP - DH, HB), 0)
                pad = jnp.where(r4 == 0, 1.0, 0.0)
                for h in range(H):
                    blk = jnp.concatenate([v[h * DH:(h + 1) * DH], pad], axis=0)
                    vt_sc[h * HP // 2:(h + 1) * HP // 2, c0:c0 + HB] = _pk(blk.astype(BF))
                qt_sc[QH // 2:D // 2, c0:c0 + HB] = _pk((v[D:MH] * qscale).astype(BF))

            def proj(c, part):
                r0 = c * D
                b1j = lambda j, n=KH: s_sc[r0:r0 + n, j * HB:(j + 1) * HB]
                b2j = lambda j: s_sc[r0 + KH:r0 + D, j * HB:(j + 1) * HB]

                def addpad(x, y, sign):
                    top = x[0:K2] + y if sign > 0 else x[0:K2] - y
                    return jnp.concatenate([top, x[K2:KH]], axis=0)
                PA0, PA1 = s_sc.at[R_A:R_A + MH, 0:HB], s_sc.at[R_A:R_A + MH, HB:RC]
                PB0, PB1 = s_sc.at[R_B:R_B + MH, 0:HB], s_sc.at[R_B:R_B + MH, HB:RC]

                def mm(lhs, rhs):
                    m = _dot(_up(lhs), rhs.astype(BF))
                    for rr in range(0, MH, TS):
                        ctoks[c].append(m[rr:rr + 8, 0:128])
                        toks.append(m[rr:rr + 8, 0:128])
                    return m
                for p in part:
                    if p == 4:
                        PA0[...] = mm(wrows(1, slice(KH, D)), b2j(0) - b1j(0, K2))
                    elif p == 7:
                        PB0[...] = PA0[...] + mm(wq_sc[4, :, 0:K2], b2j(0) + b2j(1))
                    elif p == 3:
                        PA1[...] = mm(wrows(0, slice(0, KH)), addpad(b1j(1), b2j(1), -1))
                    elif p == 2:
                        m2 = mm(wq_sc[1], b1j(0))
                        fin_bot(c, 0, m2 + PA0[...])
                        PB1[...] = PA1[...] - m2
                    elif p == 5:
                        m5 = mm(wq_sc[2, :, 0:K2], b2j(1))
                        fin_top(c, 1, PA1[...] + m5)
                        PB0[...] = PB0[...] - m5
                    elif p == 1:
                        m1 = mm(wq_sc[0], addpad(b1j(0), b2j(1), 1))
                        fin_top(c, 0, PB0[...] + m1)
                        PB1[...] = PB1[...] + m1
                    else:
                        fin_bot(c, 1, PB1[...] + mm(wq_sc[3], b1j(0) + b1j(1)))

            with scope('wait0'):
                cp_x0.wait()
            ln1(0)
            with scope('wait0b'):
                cp_wb.wait()
            wt_sc[:, KH:D] = _pk(wqkv[KH:D, :].T)
            wq_combo7()
            proj(0, [4])
            with scope('wait0c'):
                cp_wa.wait()
            if not EARLY:
                cp_wo.start(); cp_w1.start(); cp_w2.start(); cp_b1.start(); cp_b2.start()
            zpad = jnp.zeros((HP - DH, D), F32)
            wt_sc[:, 0:KH] = _pk(wqkv[0:KH, :].T)
            na = len(ctoks[0])
            proj(0, [7, 3])
            nb_ = len(ctoks[0])
            wq_combos(ctoks[0][na + int((nb_ - na) * WQ0):na + int((nb_ - na) * WQ1)] if WQT else None)
            proj(0, [5, 2])
            with scope('wait1'):
                cp_x1.wait()
            n0 = len(ctoks[0])
            proj(0, [1, 6])
            ln1(1, ctoks[0][n0:n0 + (len(ctoks[0]) - n0) * 3 // 4])
            order = [4, 7, 3, 2, 5, 1, 6]
            proj(1, order)
            n1 = len(ctoks[1])
            ln1(2, ctoks[1][0:n1 * 6 // 10])
            proj(2, order[:NPRE])
            tk3 = ctoks[1][n1 * 6 // 10:] + ctoks[2]
            ln1(3, tk3[:len(tk3) * 9 // 10])
            with scope('wait2'):
                cp_wo.wait(); cp_w1.wait(); cp_w2.wait(); cp_b1.wait(); cp_b2.wait()
            del toks[:]
            proj(2, order[NPRE:])
            proj(3, order)
            tmp_sc[...] = wo[...].astype(F32)
            blks = []
            for h in range(H):
                blks.append(tmp_sc[h * DH:(h + 1) * DH, :])
                blks.append(zpad)
            wot_sc[...] = _pk(jnp.concatenate(blks, axis=0).astype(BF).T)
            rpad = lax.broadcasted_iota(jnp.int32, (DA - D, F), 0)
            b1 = b1v[...].astype(F32).reshape(1, F)
            w1a[D:DA, :] = jnp.where(rpad == 0, b1, 0.0).astype(BF)
            FH, KH, DH2 = F // 2, DA // 2, D // 2
            p1 = [(cb, kb) for cb in range(FH // 128) for kb in range(KH // 128)]
            for pi, (cb, kb) in enumerate(p1):
                def q(i, j):
                    v = w1a[j * KH + kb * 128:j * KH + (kb + 1) * 128, i * FH + cb * 128:i * FH + (cb + 1) * 128].astype(F32)
                    if W1T and i == j:
                        v = tie(v, toks[int(pi * len(toks) * W1F) // len(p1)])
                    return v
                for n, a in enumerate(_acombos(q(0, 0), q(0, 1), q(1, 0), q(1, 1))):
                    w1s_sc[n, cb * 64:(cb + 1) * 64, kb * 128:(kb + 1) * 128] = _pk(a.astype(BF).T)
            pieces = [(rb, cb) for cb in range(FH // 128) for rb in range(DH2 // WB)]
            for pi, (rb, cb) in enumerate(pieces):
                def q(i, j):
                    v = w2t[i * DH2 + rb * WB:i * DH2 + (rb + 1) * WB, j * FH + cb * 128:j * FH + (cb + 1) * 128].astype(F32)
                    if TOK and i == j:
                        v = tie(v, toks[(pi * len(toks)) // len(pieces)])
                    return v
                for n, a in enumerate(_acombos(q(0, 0), q(0, 1), q(1, 0), q(1, 1))):
                    w2s_sc[n, rb * WB // 2:(rb + 1) * WB // 2, cb * 128:(cb + 1) * 128] = _pk(a.astype(BF))
            b2 = b2v[...].astype(F32).reshape(1, D)
            b2c_sc[...] = jnp.broadcast_to(b2, (128, D)).T

        with scope('headA'):
            m = run([None] + list(range(NA)), list(range(NA + 1)), None)

        def body(i, m):
            h = NA + UH * i
            return run([h + u for u in range(UH)], [h + u + 1 for u in range(UH)], m)
        with scope('headloop'):
            m = lax.fori_loop(0, NIT, body, m)

        TB = TQ // NB
        KS = DP - 128
        RB = 64
        NRB = D // RB
        part = {}

        def wo_part(b, rb):
            part[(b, rb)] = _dot(_up(wot_sc[rb * RB // 2:(rb + 1) * RB // 2, 0:KS]), _up(ot_sc[0:KS // 2, b * TB:(b + 1) * TB]))

        if TAIL == 0:
            run([H - 1], [None], m)
            att = [_dot(_up(wot_sc[...]), _up(ot_sc[:, b * TB:(b + 1) * TB])) for b in range(NB)]
        else:
            todo = [(b, rb) for b in range(NB) for rb in range(NRB)]

            def filler(n):
                if n % FILL == 0 and len(todo) > NRB * NB // 2 - EXTRA:
                    wo_part(*todo.pop(0))
            run([H - 1], [None], m, filler)
            while len(todo) > NRB * NB // 2 - HOLD and todo:
                wo_part(*todo.pop(0))
            att = []
            for b in range(NB):
                while todo and todo[0][0] <= b:
                    wo_part(*todo.pop(0))
                lastk = _dot(_up(wot_sc[:, KS:DP]), _up(ot_sc[KS // 2:DP // 2, b * TB:(b + 1) * TB]))
                att.append(jnp.concatenate([part[(b, rb)] for rb in range(NRB)], axis=0) + lastk)

        assert NB == 2
        KH, DH2 = DA // 2, D // 2
        rp = lax.broadcasted_iota(jnp.int32, (DA - D, TB), 0)
        ones_rows = jnp.where(rp == 0, 1.0, 0.0)
        b2c = jnp.concatenate([b2c_sc[...]] * (TB // 128), axis=1)
        FH = F // 2
        R_P, R_C, R_H = 2 * FH, 3 * FH, 4 * FH
        reg = lambda r0, n, j: s_sc.at[r0:r0 + n, j * TB:(j + 1) * TB]
        U = lambda i, j: reg(i * FH, FH, j)
        P2, P4, C11, C22 = reg(R_P, FH, 0), reg(R_P, FH, 1), reg(R_C, FH, 0), reg(R_C, FH, 1)
        R_N = R_H
        s1s = []
        for b in range(NB):
            x = xt[:, pl.ds(q0 + b * TB, TB)].astype(F32)
            h1 = x + att[b]
            h_sc[b][...] = h1
            s1s.append(jnp.sum(h1.reshape(D // 8, 8, TB), axis=0))
            s_sc[R_N + D:R_N + DA, b * TB:(b + 1) * TB] = ones_rows

        def ln2(b, tk):
            it = spread(tk, (TB // 128) * 2 * (D // LB))
            for j in range(TB // 128):
                def rd(p, r0, n):
                    return h_sc[b][pl.ds(pl.multiple_of(r0 + zs[p - 1], 8), n), j * 128:(j + 1) * 128]

                def put(r0, n, y):
                    s_sc[R_N + r0:R_N + r0 + n, b * TB + j * 128:b * TB + (j + 1) * 128] = y
                ln_paced(rd, put, it, s1s[b][:, j * 128:(j + 1) * 128])
        bq = lambda i, j: s_sc[R_N + (i - 1) * KH:R_N + i * KH, (j - 1) * TB:j * TB]
        mm1 = lambda n, v: _dot(_up(w1s_sc[n - 1]), v.astype(BF))
        act = lambda z: jnp.square(jnp.maximum(z, 0.0))
        ln2(0, None)
        m2 = mm1(2, bq(1, 1))
        P2[...] = m2
        ln2(1, [m2[rr:rr + 8, 0:128] for rr in range(0, FH, 32)])
        m4 = mm1(4, bq(2, 1) - bq(1, 1))
        U(1, 0)[...] = act(P2[...] + m4)
        P4[...] = m4
        m1 = mm1(1, bq(1, 1) + bq(2, 2))
        C11[...] = m1 + P4[...]
        C22[...] = m1 - P2[...]
        m5 = mm1(5, bq(2, 2))
        C11[...] = C11[...] - m5
        P4[...] = m5
        m7 = mm1(7, bq(2, 1) + bq(2, 2))
        U(0, 0)[...] = act(C11[...] + m7)
        m3 = mm1(3, bq(1, 2) - bq(2, 2))
        U(0, 1)[...] = act(m3 + P4[...])
        C22[...] = C22[...] + m3
        m6 = mm1(6, bq(1, 1) + bq(1, 2))
        U(1, 1)[...] = act(C22[...] + m6)

        mm2 = lambda n, v: _dot(_up(w2s_sc[n - 1]), v.astype(BF))

        def emit(i, j, y):
            rs = slice(i * DH2, (i + 1) * DH2)
            o_ref[rs, j * TB:(j + 1) * TB] = (h_sc[j][rs, :] + y + b2c[rs]).astype(o_ref.dtype)
        u = lambda i, j: U(i - 1, j - 1)[...]
        n4 = mm2(4, u(2, 1) - u(1, 1))
        n2 = mm2(2, u(1, 1))
        emit(1, 0, n2 + n4)
        n6 = mm2(6, u(1, 1) + u(1, 2))
        y22 = n6 - n2
        n1 = mm2(1, u(1, 1) + u(2, 2))
        y22 = y22 + n1
        y11 = n1 + n4
        n3 = mm2(3, u(1, 2) - u(2, 2))
        emit(1, 1, y22 + n3)
        n5 = mm2(5, u(2, 2))
        emit(0, 1, n3 + n5)
        y11 = y11 - n5
        n7 = mm2(7, u(2, 1) + u(2, 2))
        emit(0, 0, y11 + n7)

    def fn(A_x, A_wqkv, A_wo, B_x, B_w1, B_b1, B_w2, B_b2):
        xt = A_x.reshape(S, D).T
        w2t = B_w2.T
        anyspec = pl.BlockSpec(memory_space=pl.ANY)
        out = pl.pallas_call(
            kernel,
            grid=(NQ,),
            in_specs=[anyspec] * 7,
            out_specs=pl.BlockSpec((D, TQ), lambda t: (0, t)),
            out_shape=jax.ShapeDtypeStruct((D, S), BF),
            scratch_shapes=[
                pltpu.VMEM((D, S), BF), pltpu.VMEM((D, 3 * D), BF), pltpu.VMEM((D, D), BF),
                pltpu.VMEM((DA, F), BF), pltpu.VMEM((D, F), BF), pltpu.VMEM((F,), BF), pltpu.VMEM((D,), BF),
                pltpu.SemaphoreType.DMA((9,)),
                pltpu.VMEM((WR // 2, D), U32), pltpu.VMEM((D, D), F32), pltpu.VMEM((D // 2, DP), U32),
                pltpu.VMEM((7, F // 4, DA // 2), U32), pltpu.VMEM((7, D // 4, F // 2), U32), pltpu.VMEM((D, 128), F32), pltpu.VMEM((5, 3 * D // 4, DA // 2), U32),
                pltpu.VMEM((D // 2, S), U32), pltpu.VMEM((4, S // 2, GW), U32), pltpu.VMEM((DP // 2, S), U32),
                pltpu.VMEM((RS * KC, TQ), F32), pltpu.VMEM((DP // 2, TQ), U32),
                pltpu.VMEM((D, TQ // 2), F32), pltpu.VMEM((D, TQ // 2), F32)],
            compiler_params=pltpu.CompilerParams(dimension_semantics=("arbitrary",), vmem_limit_bytes=100 * 1024 * 1024),
        )(xt, A_wqkv, A_wo, B_w1, B_b1, w2t, B_b2)
        return out.T.reshape(1, S, D)
    return fn


_fn = _make()


@jax.jit
def pallas_sequential_preLN__mha_block__dense_activation_squared_relu__prompt_kernel(
    A_x: jax.Array,
    A_wqkv: jax.Array,
    A_wo: jax.Array,
    B_x: jax.Array,
    B_w1: jax.Array,
    B_b1: jax.Array,
    B_w2: jax.Array,
    B_b2: jax.Array,
):
    return _fn(A_x, A_wqkv, A_wo, B_x, B_w1, B_b1, B_w2, B_b2)
```

```python
import math

import jax
import jax.numpy as jnp
from jax import lax
from jax.experimental import pallas as pl
from jax.experimental.pallas import tpu as pltpu

S, D, H, DH, F = 2048, 448, 16, 28, 1792
HP = 32
DP = H * HP
GW = 4 * DH
DA = 512
EPS = 1e-5
BF, F32, U32 = jnp.bfloat16, jnp.float32, jnp.uint32

TQ = 512
TB = TQ // 2
KC = 128
NQ, NKC = S // TQ, S // KC
RS = 2 * NKC
UH = 7
NA = (H - 1) % UH
LAG = 1
LB = 64
KH = DA // 2
K2 = D - KH
QH = D // 2
MH = D + QH
FH = F // 2
QSCALE = (DH ** -0.5) * math.log2(math.e)


def _mo(x, m):
    return x if isinstance(x, int) else pl.multiple_of(x, m)


def _pk(x):
    return pltpu.bitcast(x, U32)


def _up(x):
    return pltpu.bitcast(x, BF)


def _dot(a, b):
    return jnp.dot(a, b, preferred_element_type=F32)


def _left_operands(a11, a12, a21, a22):
    return [a11 + a22, a21 + a22, a11, a22, a11 + a12, a21 - a11, a12 - a22]


def _spread(lst, n):
    if lst is None:
        return iter([None] * n)
    return iter([lst[(i * len(lst)) // n] for i in range(n)])


def _ring_offsets(n):
    if n == 1:
        return [0, 0]
    shifts = [RS // n] * n
    shifts[0] += RS - sum(shifts)
    assert all(LAG <= s <= NKC for s in shifts)
    off = [0]
    for s in shifts:
        off.append((off[-1] - s) % RS)
    assert off[-1] == 0
    return off


def _kernel(xt_hbm, wqkv_hbm, wo_hbm, w1_hbm, b1_hbm, w2t_hbm, b2_hbm, o_hbm,
            xt, wqkv, wo, w1a, w2t, b1v, b2v, sems,
            wt_sc, tmp_sc, wot_sc, w1s_sc, w2s_sc, b2c_sc, wq_sc,
            qt_sc, k_sc, vt_sc, s_sc, ot_sc, ha_sc, hb_sc, o_sc, osems):
    h_sc = (ha_sc, hb_sc)
    t = pl.program_id(0)
    q0 = pl.multiple_of(t * TQ, TQ)
    rowi = lax.broadcasted_iota(jnp.int32, (GW // 2, TQ), 0)

    zs = [jnp.minimum(t, 0) * 128, jnp.minimum(t, 0) * 256]
    always = lax.broadcasted_iota(jnp.int32, (8, 128), 1) > (t - 100)

    def tie(v, tok):
        if tok is None:
            return v
        n = v.shape[0]
        return jnp.where(always[None], v.reshape(n // 8, 8, 128), tok[None]).reshape(n, 128)

    def layernorm(rd, put, tk, s1=None):
        nb = D // LB
        if s1 is None:
            for b in range(nb):
                v = jnp.sum(tie(rd(0, b * LB, LB), next(tk)).reshape(LB // 8, 8, 128), axis=0)
                s1 = v if s1 is None else s1 + v
        m8 = jnp.broadcast_to(jnp.sum(s1, axis=0, keepdims=True) * (1.0 / D), (8, 128))
        s2 = None
        for b in range(nb):
            c = rd(1, b * LB, LB).reshape(LB // 8, 8, 128) - tie(m8, next(tk))[None]
            v = jnp.sum(c * c, axis=0)
            s2 = v if s2 is None else s2 + v
        r = lax.rsqrt(jnp.sum(s2, axis=0, keepdims=True) * (1.0 / D) + EPS)
        for b in range(nb):
            c = rd(2, b * LB, LB).reshape(LB // 8, 8, 128) - tie(m8, next(tk))[None]
            put(b * LB, LB, c.reshape(LB, 128) * r)

    def masked_q(h):
        if isinstance(h, int):
            g, j = h // 4, h % 4
        else:
            g, j = lax.shift_right_logical(h, 2), lax.bitwise_and(h, 3)
        q = qt_sc[pl.ds(_mo(g * (GW // 2), 8), GW // 2), pl.ds(q0, TQ)]
        hd = DH // 2
        return _up(jnp.where((rowi >= j * hd) & (rowi < (j + 1) * hd), q, jnp.zeros_like(q))), g

    def qk_chunk(qm, g, c, slot):
        s = _dot(_up(k_sc[g, c * KC // 2:(c + 1) * KC // 2, :]), qm)
        s_sc[slot * KC:(slot + 1) * KC, :] = s
        return jnp.max(s.reshape(KC // 8, 8, TQ), axis=0)

    def p_chunk(slot, m):
        return jnp.exp2(s_sc[slot * KC:(slot + 1) * KC, :] - m).astype(BF)

    def pv_chunk(h, c, p):
        v = _up(vt_sc[pl.ds(_mo(h * (HP // 2), HP // 2), HP // 2), c * KC:(c + 1) * KC])
        return _dot(v, p)

    def finish(h, o):
        l = o[0:1, :]
        r = pl.reciprocal(l, approx=True)
        r = r * (2.0 - l * r)
        ot_sc[pl.ds(_mo(h * (HP // 2), HP // 2), HP // 2), :] = _pk((o * r).astype(BF))

    def run_stages(cur, nxt, m0, filler=None):
        n_st = len(nxt)
        off = _ring_offsets(n_st)
        ms = {0: m0}
        mrun, oacc, qms, pv_at = {}, {}, {}, {}
        for j in range(n_st * NKC):
            if cur[j // NKC] is not None:
                pv_at.setdefault(j if j < NKC else j + LAG, []).append(j)
        last = max(list(pv_at) + [n_st * NKC - 1])
        for n in range(last + 1):
            ps = []
            for j in pv_at.get(n, []):
                u, c = divmod(j, NKC)
                ps.append((u, c, p_chunk((off[u] + c) % RS, ms[u])))
            if n < n_st * NKC and nxt[n // NKC] is not None:
                u, c = divmod(n, NKC)
                if c == 0:
                    qms[u] = masked_q(nxt[u])
                mc = qk_chunk(qms[u][0], qms[u][1], c, (off[u + 1] + c) % RS)
                mrun[u] = mc if c == 0 else jnp.maximum(mrun[u], mc)
                if c == NKC - 1:
                    ms[u + 1] = jnp.max(mrun[u], axis=0, keepdims=True)
            if filler is not None:
                filler(n)
            for (u, c, p) in ps:
                oc = pv_chunk(cur[u], c, p)
                oacc[u] = oc if c == 0 else oacc[u] + oc
                if c == NKC - 1:
                    finish(cur[u], oacc[u])
        return ms.get(n_st)

    @pl.when(t == 0)
    def _():
        cp_wb = pltpu.make_async_copy(wqkv_hbm.at[KH:D, :], wqkv.at[KH:D, :], sems.at[0])
        cp_wa = pltpu.make_async_copy(wqkv_hbm.at[0:KH, :], wqkv.at[0:KH, :], sems.at[1])
        cp_x0 = pltpu.make_async_copy(xt_hbm.at[:, 0:TQ], xt.at[:, 0:TQ], sems.at[2])
        cp_x1 = pltpu.make_async_copy(xt_hbm.at[:, TQ:S], xt.at[:, TQ:S], sems.at[3])
        rest = [pltpu.make_async_copy(wo_hbm, wo, sems.at[4]),
                pltpu.make_async_copy(w1_hbm, w1a.at[0:D, :], sems.at[5]),
                pltpu.make_async_copy(w2t_hbm, w2t, sems.at[6]),
                pltpu.make_async_copy(b1_hbm, b1v, sems.at[7]),
                pltpu.make_async_copy(b2_hbm, b2v, sems.at[8])]
        cp_x0.start()
        cp_wb.start()
        cp_wa.start()
        cp_x1.start()

        r_a, r_b = NQ * D, NQ * D + MH
        pa0, pa1 = s_sc.at[r_a:r_a + MH, 0:TB], s_sc.at[r_a:r_a + MH, TB:TQ]
        pb0, pb1 = s_sc.at[r_b:r_b + MH, 0:TB], s_sc.at[r_b:r_b + MH, TB:TQ]
        toks = []

        def ln1(c, tk=None):
            it = _spread(tk, (TQ // 128) * 3 * (D // LB))
            for j in range(TQ // 128):
                c0 = c * TQ + j * 128

                def rd(p, r0, n):
                    cc = c0 if (p == 0 or tk is None) else pl.multiple_of(c0 + zs[p - 1], 128)
                    return xt[r0:r0 + n, pl.ds(cc, 128)].astype(F32)

                def put(r0, n, y):
                    s_sc[c * D + r0:c * D + r0 + n, j * 128:(j + 1) * 128] = y
                layernorm(rd, put, it)

        def wrows(i, lanes):
            if i == 0:
                return jnp.concatenate([wt_sc[D // 2:D, lanes], wt_sc[0:QH // 2, lanes]], axis=0)
            return jnp.concatenate([wt_sc[D:3 * D // 2, lanes], wt_sc[QH // 2:D // 2, lanes]], axis=0)

        def wblk(i, r, lanes):
            if r < D // 2:
                r0 = (i + 1) * (D // 2) + r
            else:
                r0 = i * (QH // 2) + r - D // 2
            return _up(wt_sc[r0:r0 + 16, lanes]).astype(F32)

        def wq_operand7():
            for r in range(0, MH // 2, 16):
                v = wblk(0, r, slice(KH, D)) - wblk(1, r, slice(KH, D))
                wq_sc[4, r:r + 16, 0:K2] = _pk(v.astype(BF))

        def wq_operands(tk):
            it = _spread(tk, 2 * (MH // 32))
            z = jnp.zeros((32, KH - K2), F32)
            for r in range(0, MH // 2, 16):
                for lt in range(2):
                    tok = next(it)
                    ls = slice(lt * 128, (lt + 1) * 128)
                    a11, a21 = tie(wblk(0, r, ls), tok), tie(wblk(1, r, ls), tok)
                    if lt == 0:
                        a12, a22 = wblk(0, r, slice(KH, KH + 128)), wblk(1, r, slice(KH, KH + 128))
                    else:
                        a12 = jnp.concatenate([wblk(0, r, slice(KH + 128, D)), z], axis=1)
                        a22 = jnp.concatenate([wblk(1, r, slice(KH + 128, D)), z], axis=1)
                    for n, v in enumerate([a11 + a22, a21 + a22, a11 + a12, a21 - a11]):
                        wq_sc[n, r:r + 16, ls] = _pk(v.astype(BF))

        def fin_top(c, j, v):
            c0 = c * TQ + j * TB
            for g in range(4):
                k_sc[g, c0 // 2:(c0 + TB) // 2, :] = _pk(v[g * GW:(g + 1) * GW].astype(BF).T)
            qt_sc[0:QH // 2, c0:c0 + TB] = _pk((v[D:MH] * QSCALE).astype(BF))

        def fin_bot(c, j, v):
            c0 = c * TQ + j * TB
            r4 = lax.broadcasted_iota(jnp.int32, (HP - DH, TB), 0)
            pad = jnp.where(r4 == 0, 1.0, 0.0)
            for h in range(H):
                blk = jnp.concatenate([pad, v[h * DH:(h + 1) * DH]], axis=0)
                vt_sc[h * HP // 2:(h + 1) * HP // 2, c0:c0 + TB] = _pk(blk.astype(BF))
            qt_sc[QH // 2:D // 2, c0:c0 + TB] = _pk((v[D:MH] * QSCALE).astype(BF))

        def proj(c, products):
            r0 = c * D
            b1j = lambda j, n=KH: s_sc[r0:r0 + n, j * TB:(j + 1) * TB]
            b2j = lambda j: s_sc[r0 + KH:r0 + D, j * TB:(j + 1) * TB]

            def addpad(x, y, sign):
                top = x[0:K2] + y if sign > 0 else x[0:K2] - y
                return jnp.concatenate([top, x[K2:KH]], axis=0)

            def mm(lhs, rhs):
                m = _dot(_up(lhs), rhs.astype(BF))
                toks.extend(m[rr:rr + 8, 0:128] for rr in range(0, m.shape[0], 32))
                return m
            for p in products:
                if p == 4:
                    pa0[...] = mm(wrows(1, slice(KH, D)), b2j(0) - b1j(0, K2))
                elif isinstance(p, tuple):
                    lo, hi = p
                    pb0[lo:hi, :] = pa0[lo:hi, :] + mm(wq_sc[4, lo // 2:hi // 2, 0:K2], b2j(0) + b2j(1))
                elif p == 3:
                    pa1[...] = mm(wrows(0, slice(0, KH)), addpad(b1j(1), b2j(1), -1))
                elif p == 2:
                    m2 = mm(wq_sc[1], b1j(0))
                    fin_bot(c, 0, m2 + pa0[...])
                    pb1[...] = pa1[...] - m2
                elif p == 5:
                    m5 = mm(wq_sc[2, :, 0:K2], b2j(1))
                    fin_top(c, 1, pa1[...] + m5)
                    pb0[...] = pb0[...] - m5
                elif p == 1:
                    m1 = mm(wq_sc[0], addpad(b1j(0), b2j(1), 1))
                    fin_top(c, 0, pb0[...] + m1)
                    pb1[...] = pb1[...] + m1
                else:
                    fin_bot(c, 1, pb1[...] + mm(wq_sc[3], b1j(0) + b1j(1)))

        def take_tokens(lo=0.0, hi=1.0):
            out = toks[int(len(toks) * lo):int(len(toks) * hi)]
            del toks[:]
            return out

        m7a = 416
        cp_x0.wait()
        ln1(0)
        cp_wb.wait()
        wt_sc[:, KH:D] = _pk(wqkv[KH:D, :].T)
        wq_operand7()
        proj(0, [4, (0, m7a)])
        cp_wa.wait()
        for cp in rest:
            cp.start()
        wt_sc[:, 0:KH] = _pk(wqkv[0:KH, :].T)
        take_tokens()
        proj(0, [(m7a, MH), 3])
        wq_operands(take_tokens(0.1, 0.9))
        proj(0, [5, 2])
        cp_x1.wait()
        take_tokens()
        proj(0, [1, 6])
        ln1(1, take_tokens(0.0, 0.75))
        order = [4, (0, MH), 3, 2, 5, 1, 6]
        proj(1, order)
        n1 = len(toks) * 6 // 10
        ln1(2, toks[0:n1])
        del toks[:n1]
        proj(2, order[:2])
        ln1(3, take_tokens(0.0, 0.9))
        for cp in rest:
            cp.wait()
        proj(2, order[2:])
        proj(3, order)

        tmp_sc[...] = wo[...].astype(F32)
        zpad = jnp.zeros((HP - DH, D), F32)
        blks = []
        for h in range(H):
            blks.append(zpad)
            blks.append(tmp_sc[h * DH:(h + 1) * DH, :])
        wot_sc[...] = _pk(jnp.concatenate(blks, axis=0).astype(BF).T)
        rpad = lax.broadcasted_iota(jnp.int32, (DA - D, F), 0)
        w1a[D:DA, :] = jnp.where(rpad == 0, b1v[...].astype(F32).reshape(1, F), 0.0).astype(BF)
        it = _spread(toks[:len(toks) * 9 // 10], (FH // 128) * (KH // 128))
        for cb in range(FH // 128):
            for kb in range(KH // 128):
                tok = next(it)

                def q1(i, j):
                    v = w1a[j * KH + kb * 128:j * KH + (kb + 1) * 128,
                            i * FH + cb * 128:i * FH + (cb + 1) * 128].astype(F32)
                    return tie(v, tok) if i == j else v
                for n, a in enumerate(_left_operands(q1(0, 0), q1(0, 1), q1(1, 0), q1(1, 1))):
                    w1s_sc[n, cb * 64:(cb + 1) * 64, kb * 128:(kb + 1) * 128] = _pk(a.astype(BF).T)
        wb = 32
        it = _spread(toks, (FH // 128) * (QH // wb))
        for cb in range(FH // 128):
            for rb in range(QH // wb):
                tok = next(it)

                def q2(i, j):
                    v = w2t[i * QH + rb * wb:i * QH + (rb + 1) * wb,
                            j * FH + cb * 128:j * FH + (cb + 1) * 128].astype(F32)
                    return tie(v, tok) if i == j else v
                for n, a in enumerate(_left_operands(q2(0, 0), q2(0, 1), q2(1, 0), q2(1, 1))):
                    w2s_sc[n, rb * wb // 2:(rb + 1) * wb // 2, cb * 128:(cb + 1) * 128] = _pk(a.astype(BF))
        b2c_sc[...] = jnp.broadcast_to(b2v[...].astype(F32).reshape(1, D), (128, D)).T

    m = run_stages([None] + list(range(NA)), list(range(NA + 1)), None)

    def body(i, m):
        h = NA + UH * i
        return run_stages([h + u for u in range(UH)], [h + u + 1 for u in range(UH)], m)
    m = lax.fori_loop(0, (H - 1) // UH, body, m)

    def out_copy(i, j, qoff):
        return pltpu.make_async_copy(
            o_sc.at[i * QH:(i + 1) * QH, j * TB:(j + 1) * TB],
            o_hbm.at[i * QH:(i + 1) * QH, pl.ds(pl.multiple_of(qoff + j * TB, TB), TB)],
            osems.at[2 * i + j])

    @pl.when(t > 0)
    def _():
        for i in range(2):
            for j in range(2):
                out_copy(i, j, q0 - TQ).wait()

    ks = DP - 128
    rb_ = 64
    nrb = D // rb_
    part = {}
    todo = [(b, rb) for b in range(2) for rb in range(nrb)]

    def wo_part():
        b, rb = todo.pop(0)
        part[(b, rb)] = _dot(_up(wot_sc[rb * rb_ // 2:(rb + 1) * rb_ // 2, 0:ks]),
                             _up(ot_sc[0:ks // 2, b * TB:(b + 1) * TB]))

    def filler(n):
        if n % 2 == 0:
            wo_part()
    run_stages([H - 1], [None], m, filler)
    wo_part()
    wo_part()
    att = []
    for b in range(2):
        while todo and todo[0][0] <= b:
            wo_part()
        rhs = _up(ot_sc[ks // 2:DP // 2, b * TB:(b + 1) * TB])
        lastk = jnp.concatenate([_dot(_up(wot_sc[i * QH // 2:(i + 1) * QH // 2, ks:DP]), rhs)
                                 for i in range(2)], axis=0)
        att.append(jnp.concatenate([part[(b, rb)] for rb in range(nrb)], axis=0) + lastk)

    reg = lambda r0, j: s_sc.at[r0:r0 + FH, j * TB:(j + 1) * TB]
    act_out = lambda i, j: reg((i - 1) * FH, j - 1)
    p2, p4, c11, c22 = reg(2 * FH, 0), reg(2 * FH, 1), reg(3 * FH, 0), reg(3 * FH, 1)
    r_n = 4 * FH
    rp = lax.broadcasted_iota(jnp.int32, (DA - D, TB), 0)
    ones_rows = jnp.where(rp == 0, 1.0, 0.0)
    s1s = []
    for b in range(2):
        h1 = xt[:, pl.ds(q0 + b * TB, TB)].astype(F32) + att[b]
        h_sc[b][...] = h1
        s1s.append(jnp.sum(h1.reshape(D // 8, 8, TB), axis=0))
        s_sc[r_n + D:r_n + DA, b * TB:(b + 1) * TB] = ones_rows

    def ln2(b, tk):
        it = _spread(tk, (TB // 128) * 2 * (D // LB))
        for j in range(TB // 128):
            def rd(p, r0, n):
                return h_sc[b][pl.ds(pl.multiple_of(r0 + zs[p - 1], 8), n), j * 128:(j + 1) * 128]

            def put(r0, n, y):
                s_sc[r_n + r0:r_n + r0 + n, b * TB + j * 128:b * TB + (j + 1) * 128] = y
            layernorm(rd, put, it, s1s[b][:, j * 128:(j + 1) * 128])

    bq = lambda i, j: s_sc[r_n + (i - 1) * KH:r_n + i * KH, (j - 1) * TB:j * TB]
    mm1 = lambda n, v: _dot(_up(w1s_sc[n - 1]), v.astype(BF))
    act = lambda z: jnp.square(jnp.maximum(z, 0.0))
    ln2(0, None)
    m2 = mm1(2, bq(1, 1))
    p2[...] = m2
    ln2(1, [m2[rr:rr + 8, 0:128] for rr in range(FH // 4, FH, 16)])
    m4 = mm1(4, bq(2, 1) - bq(1, 1))
    act_out(2, 1)[...] = act(p2[...] + m4)
    p4[...] = m4
    m1 = mm1(1, bq(1, 1) + bq(2, 2))
    c11[...] = m1 + p4[...]
    c22[...] = m1 - p2[...]
    m5 = mm1(5, bq(2, 2))
    c11[...] = c11[...] - m5
    p4[...] = m5
    m7 = mm1(7, bq(2, 1) + bq(2, 2))
    act_out(1, 1)[...] = act(c11[...] + m7)
    m3 = mm1(3, bq(1, 2) - bq(2, 2))
    act_out(1, 2)[...] = act(m3 + p4[...])
    c22[...] = c22[...] + m3
    m6 = mm1(6, bq(1, 1) + bq(1, 2))
    act_out(2, 2)[...] = act(c22[...] + m6)

    mm2 = lambda n, v: _dot(_up(w2s_sc[n - 1]), v.astype(BF))
    u = lambda i, j: act_out(i, j)[...]
    b2c = jnp.concatenate([b2c_sc[...]] * (TB // 128), axis=1)

    def emit(i, j, y):
        rs = slice(i * QH, (i + 1) * QH)
        o_sc[rs, j * TB:(j + 1) * TB] = (h_sc[j][rs, :] + y + b2c[rs]).astype(BF)
        out_copy(i, j, q0).start()
    n4 = mm2(4, u(2, 1) - u(1, 1))
    n2 = mm2(2, u(1, 1))
    emit(1, 0, n2 + n4)
    n6 = mm2(6, u(1, 1) + u(1, 2))
    y22 = n6 - n2
    n1 = mm2(1, u(1, 1) + u(2, 2))
    y22 = y22 + n1
    y11 = n1 + n4
    n3 = mm2(3, u(1, 2) - u(2, 2))
    emit(1, 1, y22 + n3)
    n5 = mm2(5, u(2, 2))
    emit(0, 1, n3 + n5)
    y11 = y11 - n5
    n7 = mm2(7, u(2, 1) + u(2, 2))
    emit(0, 0, y11 + n7)

    @pl.when(t == NQ - 1)
    def _():
        for i in range(2):
            for j in range(2):
                out_copy(i, j, q0).wait()


@jax.jit
def pallas_sequential_preLN__mha_block__dense_activation_squared_relu__prompt_kernel(
    A_x: jax.Array,
    A_wqkv: jax.Array,
    A_wo: jax.Array,
    B_x: jax.Array,
    B_w1: jax.Array,
    B_b1: jax.Array,
    B_w2: jax.Array,
    B_b2: jax.Array,
):
    del B_x
    anyspec = pl.BlockSpec(memory_space=pl.ANY)
    out_t = pl.pallas_call(
        _kernel,
        grid=(NQ,),
        in_specs=[anyspec] * 7,
        out_specs=anyspec,
        out_shape=jax.ShapeDtypeStruct((D, S), BF),
        scratch_shapes=[
            pltpu.VMEM((D, S), BF),
            pltpu.VMEM((D, 3 * D), BF),
            pltpu.VMEM((D, D), BF),
            pltpu.VMEM((DA, F), BF),
            pltpu.VMEM((D, F), BF),
            pltpu.VMEM((F,), BF),
            pltpu.VMEM((D,), BF),
            pltpu.SemaphoreType.DMA((9,)),
            pltpu.VMEM((3 * D // 2, D), U32),
            pltpu.VMEM((D, D), F32),
            pltpu.VMEM((D // 2, DP), U32),
            pltpu.VMEM((7, FH // 2, KH), U32),
            pltpu.VMEM((7, QH // 2, FH), U32),
            pltpu.VMEM((D, 128), F32),
            pltpu.VMEM((5, MH // 2, KH), U32),
            pltpu.VMEM((D // 2, S), U32),
            pltpu.VMEM((4, S // 2, GW), U32),
            pltpu.VMEM((DP // 2, S), U32),
            pltpu.VMEM((RS * KC, TQ), F32),
            pltpu.VMEM((DP // 2, TQ), U32),
            pltpu.VMEM((D, TB), F32),
            pltpu.VMEM((D, TB), F32),
            pltpu.VMEM((D, TQ), BF),
            pltpu.SemaphoreType.DMA((4,)),
        ],
        compiler_params=pltpu.CompilerParams(dimension_semantics=("arbitrary",),
                                             vmem_limit_bytes=100 * 1024 * 1024),
    )(A_x.reshape(S, D).T, A_wqkv, A_wo, B_w1, B_b1, B_w2.T, B_b2)
    return out_t.T.reshape(1, S, D)
```

```python
import math

import jax
import jax.numpy as jnp
from jax import lax
from jax.experimental import pallas as pl
from jax.experimental.pallas import tpu as pltpu

S, D, H, DH, F = 2048, 448, 16, 28, 1792
HP = 32
DP = H * HP
GW = 4 * DH
DA = 512
EPS = 1e-5
BF, F32, U32 = jnp.bfloat16, jnp.float32, jnp.uint32

TQ = 512
TB = TQ // 2
KC = 128
NQ, NKC = S // TQ, S // KC
RS = 2 * NKC
UH = 7
NA = (H - 1) % UH
LAG = 1
LB = 32
KH = DA // 2
K2 = D - KH
QH = D // 2
MH = D + QH
FH = F // 2
QSCALE = (DH ** -0.5) * math.log2(math.e)


def _mo(x, m):
    return x if isinstance(x, int) else pl.multiple_of(x, m)


def _pk(x):
    return pltpu.bitcast(x, U32)


def _up(x):
    return pltpu.bitcast(x, BF)


def _dot(a, b):
    return jnp.dot(a, b, preferred_element_type=F32)


def _left_operands(a11, a12, a21, a22):
    return [a11 + a22, a21 + a22, a11, a22, a11 + a12, a21 - a11, a12 - a22]


def _spread(lst, n):
    if lst is None:
        return iter([None] * n)
    return iter([lst[(i * len(lst)) // n] for i in range(n)])


def _ring_offsets(n):
    if n == 1:
        return [0, 0]
    shifts = [RS // n] * n
    shifts[0] += RS - sum(shifts)
    assert all(LAG <= s <= NKC for s in shifts)
    off = [0]
    for s in shifts:
        off.append((off[-1] - s) % RS)
    assert off[-1] == 0
    return off


def _kernel(xt_hbm, wqkv_hbm, wo_hbm, w1_hbm, b1_hbm, w2t_hbm, b2_hbm, o_hbm,
            xt, wqkv, wo, w1a, w2t, b1v, b2v, sems,
            wt_sc, tmp_sc, wot_sc, w1s_sc, w2s_sc, b2c_sc, wq_sc,
            qt_sc, k_sc, vt_sc, s_sc, ot_sc, ha_sc, hb_sc, o_sc, osems):
    h_sc = (ha_sc, hb_sc)
    t = pl.program_id(0)
    q0 = pl.multiple_of(t * TQ, TQ)
    rowi = lax.broadcasted_iota(jnp.int32, (GW // 2, TQ), 0)

    zs = [jnp.minimum(t, 0) * 128, jnp.minimum(t, 0) * 256]
    always = lax.broadcasted_iota(jnp.int32, (8, 128), 1) > (t - 100)

    def tie(v, tok):
        if tok is None:
            return v
        n = v.shape[0]
        return jnp.where(always[None], v.reshape(n // 8, 8, 128), tok[None]).reshape(n, 128)

    def layernorm(rd, put, tk, s1=None):
        nb = D // LB
        if s1 is None:
            for b in range(nb):
                v = jnp.sum(tie(rd(0, b * LB, LB), next(tk)).reshape(LB // 8, 8, 128), axis=0)
                s1 = v if s1 is None else s1 + v
        m8 = jnp.broadcast_to(jnp.sum(s1, axis=0, keepdims=True) * (1.0 / D), (8, 128))
        s2 = None
        for b in range(nb):
            c = rd(1, b * LB, LB).reshape(LB // 8, 8, 128) - tie(m8, next(tk))[None]
            v = jnp.sum(c * c, axis=0)
            s2 = v if s2 is None else s2 + v
        r = lax.rsqrt(jnp.sum(s2, axis=0, keepdims=True) * (1.0 / D) + EPS)
        for b in range(nb):
            c = rd(2, b * LB, LB).reshape(LB // 8, 8, 128) - tie(m8, next(tk))[None]
            put(b * LB, LB, c.reshape(LB, 128) * r)

    def masked_q(h):
        if isinstance(h, int):
            g, j = h // 4, h % 4
        else:
            g, j = lax.shift_right_logical(h, 2), lax.bitwise_and(h, 3)
        q = qt_sc[pl.ds(_mo(g * (GW // 2), 8), GW // 2), pl.ds(q0, TQ)]
        hd = DH // 2
        return _up(jnp.where((rowi >= j * hd) & (rowi < (j + 1) * hd), q, jnp.zeros_like(q))), g

    def qk_chunk(qm, g, c, slot):
        s = _dot(_up(k_sc[g, c * KC // 2:(c + 1) * KC // 2, :]), qm)
        s_sc[slot * KC:(slot + 1) * KC, :] = s
        return jnp.max(s.reshape(KC // 8, 8, TQ), axis=0)

    def p_chunk(slot, m):
        return jnp.exp2(s_sc[slot * KC:(slot + 1) * KC, :] - m).astype(BF)

    def pv_chunk(h, c, p):
        v = _up(vt_sc[pl.ds(_mo(h * (HP // 2), HP // 2), HP // 2), c * KC:(c + 1) * KC])
        return _dot(v, p)

    def finish(h, o):
        l = o[0:1, :]
        r = pl.reciprocal(l, approx=True)
        r = r * (2.0 - l * r)
        ot_sc[pl.ds(_mo(h * (HP // 2), HP // 2), HP // 2), :] = _pk((o * r).astype(BF))

    def run_stages(cur, nxt, m0, filler=None):
        n_st = len(nxt)
        off = _ring_offsets(n_st)
        ms = {0: m0}
        mrun, oacc, qms, pv_at = {}, {}, {}, {}
        for j in range(n_st * NKC):
            if cur[j // NKC] is not None:
                pv_at.setdefault(j if j < NKC else j + LAG, []).append(j)
        last = max(list(pv_at) + [n_st * NKC - 1])
        for n in range(last + 1):
            ps = []
            for j in pv_at.get(n, []):
                u, c = divmod(j, NKC)
                ps.append((u, c, p_chunk((off[u] + c) % RS, ms[u])))
            if n < n_st * NKC and nxt[n // NKC] is not None:
                u, c = divmod(n, NKC)
                if c == 0:
                    qms[u] = masked_q(nxt[u])
                mc = qk_chunk(qms[u][0], qms[u][1], c, (off[u + 1] + c) % RS)
                mrun[u] = mc if c == 0 else jnp.maximum(mrun[u], mc)
                if c == NKC - 1:
                    ms[u + 1] = jnp.max(mrun[u], axis=0, keepdims=True)
            if filler is not None:
                filler(n)
            for (u, c, p) in ps:
                oc = pv_chunk(cur[u], c, p)
                oacc[u] = oc if c == 0 else oacc[u] + oc
                if c == NKC - 1:
                    finish(cur[u], oacc[u])
        return ms.get(n_st)

    @pl.when(t == 0)
    def _():
        cp_wb = pltpu.make_async_copy(wqkv_hbm.at[KH:D, :], wqkv.at[KH:D, :], sems.at[0])
        cp_wa = pltpu.make_async_copy(wqkv_hbm.at[0:KH, :], wqkv.at[0:KH, :], sems.at[1])
        cp_x0 = pltpu.make_async_copy(xt_hbm.at[:, 0:TQ], xt.at[:, 0:TQ], sems.at[2])
        cp_x1 = pltpu.make_async_copy(xt_hbm.at[:, TQ:S], xt.at[:, TQ:S], sems.at[3])
        rest = [pltpu.make_async_copy(wo_hbm, wo, sems.at[4]),
                pltpu.make_async_copy(w1_hbm, w1a.at[0:D, :], sems.at[5]),
                pltpu.make_async_copy(w2t_hbm, w2t, sems.at[6]),
                pltpu.make_async_copy(b1_hbm, b1v, sems.at[7]),
                pltpu.make_async_copy(b2_hbm, b2v, sems.at[8])]
        cp_x0.start()
        cp_wb.start()
        cp_wa.start()
        cp_x1.start()

        r_a, r_b = NQ * D, NQ * D + MH
        pa0, pa1 = s_sc.at[r_a:r_a + MH, 0:TB], s_sc.at[r_a:r_a + MH, TB:TQ]
        pb0, pb1 = s_sc.at[r_b:r_b + MH, 0:TB], s_sc.at[r_b:r_b + MH, TB:TQ]
        toks = []

        def ln1(c, tk=None):
            it = _spread(tk, (TQ // 128) * 3 * (D // LB))
            for j in range(TQ // 128):
                c0 = c * TQ + j * 128

                def rd(p, r0, n):
                    cc = c0 if (p == 0 or tk is None) else pl.multiple_of(c0 + zs[p - 1], 128)
                    return xt[r0:r0 + n, pl.ds(cc, 128)].astype(F32)

                def put(r0, n, y):
                    s_sc[c * D + r0:c * D + r0 + n, j * 128:(j + 1) * 128] = y
                layernorm(rd, put, it)

        def wrows(i, lanes):
            if i == 0:
                return jnp.concatenate([wt_sc[D // 2:D, lanes], wt_sc[0:QH // 2, lanes]], axis=0)
            return jnp.concatenate([wt_sc[D:3 * D // 2, lanes], wt_sc[QH // 2:D // 2, lanes]], axis=0)

        def wblk(i, r, lanes):
            if r < D // 2:
                r0 = (i + 1) * (D // 2) + r
            else:
                r0 = i * (QH // 2) + r - D // 2
            return _up(wt_sc[r0:r0 + 16, lanes]).astype(F32)

        def wq_operand7():
            for r in range(0, MH // 2, 16):
                v = wblk(0, r, slice(KH, D)) - wblk(1, r, slice(KH, D))
                wq_sc[4, r:r + 16, 0:K2] = _pk(v.astype(BF))

        def wq_operands(tk):
            it = _spread(tk, 2 * (MH // 32))
            z = jnp.zeros((32, KH - K2), F32)
            for r in range(0, MH // 2, 16):
                for lt in range(2):
                    tok = next(it)
                    ls = slice(lt * 128, (lt + 1) * 128)
                    a11, a21 = tie(wblk(0, r, ls), tok), tie(wblk(1, r, ls), tok)
                    if lt == 0:
                        a12, a22 = wblk(0, r, slice(KH, KH + 128)), wblk(1, r, slice(KH, KH + 128))
                    else:
                        a12 = jnp.concatenate([wblk(0, r, slice(KH + 128, D)), z], axis=1)
                        a22 = jnp.concatenate([wblk(1, r, slice(KH + 128, D)), z], axis=1)
                    for n, v in enumerate([a11 + a22, a21 + a22, a11 + a12, a21 - a11]):
                        wq_sc[n, r:r + 16, ls] = _pk(v.astype(BF))

        def fin_top(c, j, v):
            c0 = c * TQ + j * TB
            for g in range(4):
                k_sc[g, c0 // 2:(c0 + TB) // 2, :] = _pk(v[g * GW:(g + 1) * GW].astype(BF).T)
            qt_sc[0:QH // 2, c0:c0 + TB] = _pk((v[D:MH] * QSCALE).astype(BF))

        def fin_bot(c, j, v):
            c0 = c * TQ + j * TB
            r4 = lax.broadcasted_iota(jnp.int32, (HP - DH, TB), 0)
            pad = jnp.where(r4 == 0, 1.0, 0.0)
            for h in range(H):
                blk = jnp.concatenate([pad, v[h * DH:(h + 1) * DH]], axis=0)
                vt_sc[h * HP // 2:(h + 1) * HP // 2, c0:c0 + TB] = _pk(blk.astype(BF))
            qt_sc[QH // 2:D // 2, c0:c0 + TB] = _pk((v[D:MH] * QSCALE).astype(BF))

        def proj(c, products):
            r0 = c * D
            b1j = lambda j, n=KH: s_sc[r0:r0 + n, j * TB:(j + 1) * TB]
            b2j = lambda j: s_sc[r0 + KH:r0 + D, j * TB:(j + 1) * TB]

            def addpad(x, y, sign):
                top = x[0:K2] + y if sign > 0 else x[0:K2] - y
                return jnp.concatenate([top, x[K2:KH]], axis=0)

            def mm(lhs, rhs):
                m = _dot(_up(lhs), rhs.astype(BF))
                toks.extend(m[rr:rr + 8, 0:128] for rr in range(0, m.shape[0], 16))
                return m
            for p in products:
                if p == 4:
                    pa0[...] = mm(wrows(1, slice(KH, D)), b2j(0) - b1j(0, K2))
                elif isinstance(p, tuple):
                    lo, hi = p
                    pb0[lo:hi, :] = pa0[lo:hi, :] + mm(wq_sc[4, lo // 2:hi // 2, 0:K2], b2j(0) + b2j(1))
                elif p == 3:
                    pa1[...] = mm(wrows(0, slice(0, KH)), addpad(b1j(1), b2j(1), -1))
                elif p == 2:
                    m2 = mm(wq_sc[1], b1j(0))
                    fin_bot(c, 0, m2 + pa0[...])
                    pb1[...] = pa1[...] - m2
                elif p == 5:
                    m5 = mm(wq_sc[2, :, 0:K2], b2j(1))
                    fin_top(c, 1, pa1[...] + m5)
                    pb0[...] = pb0[...] - m5
                elif p == 1:
                    m1 = mm(wq_sc[0], addpad(b1j(0), b2j(1), 1))
                    fin_top(c, 0, pb0[...] + m1)
                    pb1[...] = pb1[...] + m1
                else:
                    fin_bot(c, 1, pb1[...] + mm(wq_sc[3], b1j(0) + b1j(1)))

        def take_tokens(lo=0.0, hi=1.0):
            out = toks[int(len(toks) * lo):int(len(toks) * hi)]
            del toks[:]
            return out

        m7a = 416
        cp_x0.wait()
        ln1(0)
        cp_wb.wait()
        wt_sc[:, KH:D] = _pk(wqkv[KH:D, :].T)
        wq_operand7()
        proj(0, [4, (0, m7a)])
        cp_wa.wait()
        for cp in rest:
            cp.start()
        wt_sc[:, 0:KH] = _pk(wqkv[0:KH, :].T)
        take_tokens()
        proj(0, [(m7a, MH), 3])
        wq_operands(take_tokens(0.1, 0.9))
        proj(0, [5, 2])
        cp_x1.wait()
        take_tokens()
        proj(0, [1, 6])
        ln1(1, take_tokens(0.0, 0.85))
        order = [4, (0, MH), 3, 2, 5, 1, 6]
        proj(1, order)
        n1 = len(toks) * 6 // 10
        ln1(2, toks[0:n1])
        del toks[:n1]
        proj(2, order[:2])
        ln1(3, take_tokens(0.0, 0.9))
        for cp in rest:
            cp.wait()
        proj(2, order[2:])
        proj(3, order)

        tmp_sc[...] = wo[...].astype(F32)
        zpad = jnp.zeros((HP - DH, D), F32)
        blks = []
        for h in range(H):
            blks.append(zpad)
            blks.append(tmp_sc[h * DH:(h + 1) * DH, :])
        wot_sc[...] = _pk(jnp.concatenate(blks, axis=0).astype(BF).T)
        rpad = lax.broadcasted_iota(jnp.int32, (DA - D, F), 0)
        w1a[D:DA, :] = jnp.where(rpad == 0, b1v[...].astype(F32).reshape(1, F), 0.0).astype(BF)
        it = _spread(toks[len(toks) // 20:len(toks) * 9 // 10], (FH // 128) * (KH // 128))
        for cb in range(FH // 128):
            for kb in range(KH // 128):
                tok = next(it)

                def q1(i, j):
                    v = w1a[j * KH + kb * 128:j * KH + (kb + 1) * 128,
                            i * FH + cb * 128:i * FH + (cb + 1) * 128].astype(F32)
                    return tie(v, tok) if i == j else v
                for n, a in enumerate(_left_operands(q1(0, 0), q1(0, 1), q1(1, 0), q1(1, 1))):
                    w1s_sc[n, cb * 64:(cb + 1) * 64, kb * 128:(kb + 1) * 128] = _pk(a.astype(BF).T)
        wb = 32
        it = _spread(toks, (FH // 128) * (QH // wb))
        for cb in range(FH // 128):
            for rb in range(QH // wb):
                tok = next(it)

                def q2(i, j):
                    v = w2t[i * QH + rb * wb:i * QH + (rb + 1) * wb,
                            j * FH + cb * 128:j * FH + (cb + 1) * 128].astype(F32)
                    return tie(v, tok) if i == j else v
                for n, a in enumerate(_left_operands(q2(0, 0), q2(0, 1), q2(1, 0), q2(1, 1))):
                    w2s_sc[n, rb * wb // 2:(rb + 1) * wb // 2, cb * 128:(cb + 1) * 128] = _pk(a.astype(BF))
        b2c_sc[...] = jnp.broadcast_to(b2v[...].astype(F32).reshape(1, D), (128, D)).T

    m = run_stages([None] + list(range(NA)), list(range(NA + 1)), None)

    def body(i, m):
        h = NA + UH * i
        return run_stages([h + u for u in range(UH)], [h + u + 1 for u in range(UH)], m)
    m = lax.fori_loop(0, (H - 1) // UH, body, m)

    def out_copy(i, j, qoff):
        return pltpu.make_async_copy(
            o_sc.at[i * QH:(i + 1) * QH, j * TB:(j + 1) * TB],
            o_hbm.at[i * QH:(i + 1) * QH, pl.ds(pl.multiple_of(qoff + j * TB, TB), TB)],
            osems.at[2 * i + j])

    @pl.when(t > 0)
    def _():
        for i in range(2):
            for j in range(2):
                out_copy(i, j, q0 - TQ).wait()

    ks = DP - 128
    rb_ = 64
    nrb = D // rb_
    part = {}
    todo = [(b, rb) for b in range(2) for rb in range(nrb)]

    def wo_part():
        b, rb = todo.pop(0)
        part[(b, rb)] = _dot(_up(wot_sc[rb * rb_ // 2:(rb + 1) * rb_ // 2, 0:ks]),
                             _up(ot_sc[0:ks // 2, b * TB:(b + 1) * TB]))

    def filler(n):
        if n % 2 == 0:
            wo_part()
    run_stages([H - 1], [None], m, filler)
    wo_part()
    wo_part()
    att = []
    for b in range(2):
        while todo and todo[0][0] <= b:
            wo_part()
        rhs = _up(ot_sc[ks // 2:DP // 2, b * TB:(b + 1) * TB])
        lastk = jnp.concatenate([_dot(_up(wot_sc[i * QH // 2:(i + 1) * QH // 2, ks:DP]), rhs)
                                 for i in range(2)], axis=0)
        att.append(jnp.concatenate([part[(b, rb)] for rb in range(nrb)], axis=0) + lastk)

    reg = lambda r0, j: s_sc.at[r0:r0 + FH, j * TB:(j + 1) * TB]
    act_out = lambda i, j: reg((i - 1) * FH, j - 1)
    p2, p4, c11, c22 = reg(2 * FH, 0), reg(2 * FH, 1), reg(3 * FH, 0), reg(3 * FH, 1)
    r_n = 4 * FH
    rp = lax.broadcasted_iota(jnp.int32, (DA - D, TB), 0)
    ones_rows = jnp.where(rp == 0, 1.0, 0.0)
    s1s = []
    for b in range(2):
        h1 = xt[:, pl.ds(q0 + b * TB, TB)].astype(F32) + att[b]
        h_sc[b][...] = h1
        s1s.append(jnp.sum(h1.reshape(D // 8, 8, TB), axis=0))
        s_sc[r_n + D:r_n + DA, b * TB:(b + 1) * TB] = ones_rows

    def ln2(b, tk):
        it = _spread(tk, (TB // 128) * 2 * (D // LB))
        for j in range(TB // 128):
            def rd(p, r0, n):
                return h_sc[b][pl.ds(pl.multiple_of(r0 + zs[p - 1], 8), n), j * 128:(j + 1) * 128]

            def put(r0, n, y):
                s_sc[r_n + r0:r_n + r0 + n, b * TB + j * 128:b * TB + (j + 1) * 128] = y
            layernorm(rd, put, it, s1s[b][:, j * 128:(j + 1) * 128])

    bq = lambda i, j: s_sc[r_n + (i - 1) * KH:r_n + i * KH, (j - 1) * TB:j * TB]
    mm1 = lambda n, v: _dot(_up(w1s_sc[n - 1]), v.astype(BF))
    act = lambda z: jnp.square(jnp.maximum(z, 0.0))
    ln2(0, None)
    m2 = mm1(2, bq(1, 1))
    p2[...] = m2
    ln2(1, [m2[rr:rr + 8, 0:128] for rr in range(FH // 4, FH, 16)])
    m4 = mm1(4, bq(2, 1) - bq(1, 1))
    act_out(2, 1)[...] = act(p2[...] + m4)
    p4[...] = m4
    m1 = mm1(1, bq(1, 1) + bq(2, 2))
    c11[...] = m1 + p4[...]
    c22[...] = m1 - p2[...]
    m5 = mm1(5, bq(2, 2))
    c11[...] = c11[...] - m5
    p4[...] = m5
    m7 = mm1(7, bq(2, 1) + bq(2, 2))
    act_out(1, 1)[...] = act(c11[...] + m7)
    m3 = mm1(3, bq(1, 2) - bq(2, 2))
    act_out(1, 2)[...] = act(m3 + p4[...])
    c22[...] = c22[...] + m3
    m6 = mm1(6, bq(1, 1) + bq(1, 2))
    act_out(2, 2)[...] = act(c22[...] + m6)

    mm2 = lambda n, v: _dot(_up(w2s_sc[n - 1]), v.astype(BF))
    u = lambda i, j: act_out(i, j)[...]
    b2c = jnp.concatenate([b2c_sc[...]] * (TB // 128), axis=1)

    def emit(i, j, y):
        rs = slice(i * QH, (i + 1) * QH)
        o_sc[rs, j * TB:(j + 1) * TB] = (h_sc[j][rs, :] + y + b2c[rs]).astype(BF)
        out_copy(i, j, q0).start()
    n4 = mm2(4, u(2, 1) - u(1, 1))
    n2 = mm2(2, u(1, 1))
    emit(1, 0, n2 + n4)
    n6 = mm2(6, u(1, 1) + u(1, 2))
    y22 = n6 - n2
    n1 = mm2(1, u(1, 1) + u(2, 2))
    y22 = y22 + n1
    y11 = n1 + n4
    n3 = mm2(3, u(1, 2) - u(2, 2))
    emit(1, 1, y22 + n3)
    n5 = mm2(5, u(2, 2))
    emit(0, 1, n3 + n5)
    y11 = y11 - n5
    n7 = mm2(7, u(2, 1) + u(2, 2))
    emit(0, 0, y11 + n7)

    @pl.when(t == NQ - 1)
    def _():
        for i in range(2):
            for j in range(2):
                out_copy(i, j, q0).wait()


@jax.jit
def pallas_sequential_preLN__mha_block__dense_activation_squared_relu__prompt_kernel(
    A_x: jax.Array,
    A_wqkv: jax.Array,
    A_wo: jax.Array,
    B_x: jax.Array,
    B_w1: jax.Array,
    B_b1: jax.Array,
    B_w2: jax.Array,
    B_b2: jax.Array,
):
    del B_x
    anyspec = pl.BlockSpec(memory_space=pl.ANY)
    out_t = pl.pallas_call(
        _kernel,
        grid=(NQ,),
        in_specs=[anyspec] * 7,
        out_specs=anyspec,
        out_shape=jax.ShapeDtypeStruct((D, S), BF),
        scratch_shapes=[
            pltpu.VMEM((D, S), BF),
            pltpu.VMEM((D, 3 * D), BF),
            pltpu.VMEM((D, D), BF),
            pltpu.VMEM((DA, F), BF),
            pltpu.VMEM((D, F), BF),
            pltpu.VMEM((F,), BF),
            pltpu.VMEM((D,), BF),
            pltpu.SemaphoreType.DMA((9,)),
            pltpu.VMEM((3 * D // 2, D), U32),
            pltpu.VMEM((D, D), F32),
            pltpu.VMEM((D // 2, DP), U32),
            pltpu.VMEM((7, FH // 2, KH), U32),
            pltpu.VMEM((7, QH // 2, FH), U32),
            pltpu.VMEM((D, 128), F32),
            pltpu.VMEM((5, MH // 2, KH), U32),
            pltpu.VMEM((D // 2, S), U32),
            pltpu.VMEM((4, S // 2, GW), U32),
            pltpu.VMEM((DP // 2, S), U32),
            pltpu.VMEM((RS * KC, TQ), F32),
            pltpu.VMEM((DP // 2, TQ), U32),
            pltpu.VMEM((D, TB), F32),
            pltpu.VMEM((D, TB), F32),
            pltpu.VMEM((D, TQ), BF),
            pltpu.SemaphoreType.DMA((4,)),
        ],
        compiler_params=pltpu.CompilerParams(dimension_semantics=("arbitrary",),
                                             vmem_limit_bytes=100 * 1024 * 1024),
    )(A_x.reshape(S, D).T, A_wqkv, A_wo, B_w1, B_b1, B_w2.T, B_b2)
    return out_t.T.reshape(1, S, D)
```
